```python
import os as _os
_os.environ.setdefault("JAX_PLATFORMS", "cpu")
import jax
import jax.numpy as jnp

def _softmax(x, axis=-1):
    return jax.nn.softmax(x, axis=axis)
def _gelu(x):
    return jax.nn.gelu(x, approximate=True)
def _silu(x):
    return jax.nn.silu(x)
def _sigmoid(x):
    return jax.nn.sigmoid(x)
def _layernorm(x, axis=-1, eps=1e-5):
    m = jnp.mean(x, axis=axis, keepdims=True)
    v = jnp.var(x, axis=axis, keepdims=True)
    return (x - m) / jnp.sqrt(v + eps)
def _scatter_add(tgt, idx, src, axis=0):
    return tgt.at[idx].add(src)
def _segment_sum(src, seg, n):
    return jax.ops.segment_sum(src, seg, n)
class _Rng:
    def __init__(self, key):
        self._k = key
    def _next(self):
        self._k, sub = jax.random.split(self._k)
        return sub
    def normal(self, shape):
        return jax.random.normal(self._next(), shape, dtype=jnp.bfloat16)
    def randint(self, lo, hi, shape):
        return jax.random.randint(self._next(), shape, lo, hi, dtype=jnp.int32)
    def uniform(self, shape, lo=0.0, hi=1.0):
        return jax.random.uniform(self._next(), shape, jnp.bfloat16, lo, hi)
    def permutation(self, n):
        return jax.random.permutation(self._next(), n)


kernel_name = 'concat_heads__gqa_block_cached__mha_block_cached__near_ridge'

def setup_inputs():
    _rng = _Rng(jax.random.key(int.from_bytes(__import__("os").urandom(4), "little")))
    _w = (lambda a: (lambda t: t.astype(jnp.bfloat16) if jnp.issubdtype(t.dtype, jnp.floating) else t)(jnp.asarray(a)))
    def _A_setup():
        B, Sq, D = 8, 112, 448
        Hq, Hkv, Sk, Dh = 16, 8, 512, 256
        assert Hq % Hkv == 0, (Hq, Hkv)
        return {
            "x": _w((lambda *s: _rng.normal(s) * 0.8)(B, Sq, D)),
            "k_cache": _w((lambda *s: _rng.normal(s) * 0.8)(B, Hkv, Sk, Dh)),
            "v_cache": _w((lambda *s: _rng.normal(s) * 0.05)(B, Hkv, Sk, Dh)),
            "wq": _w((lambda *s: _rng.normal(s) * 0.8)(D, Hq * Dh) * (D ** -0.5)),
            "wo": _w((lambda *s: _rng.normal(s) * 0.05)(Hq * Dh, D) * ((Hq * Dh) ** -0.5)),
        }
    _A_in = _A_setup()

    def _B_setup():
        B, Sq, D = 8, 112, 448
        H, Sk, Dh = 16, 512, 256
        return {
            "x": _w((lambda *s: _rng.normal(s) * 0.8)(B, Sq, D)),
            "k_cache": _w((lambda *s: _rng.normal(s) * 0.8)(B, H, Sk, Dh)),
            "v_cache": _w((lambda *s: _rng.normal(s) * 0.05)(B, H, Sk, Dh)),
            "wq": _w((lambda *s: _rng.normal(s) * 0.8)(D, H * Dh) * (D ** -0.5)),
            "wo": _w((lambda *s: _rng.normal(s) * 0.05)(H * Dh, D) * ((H * Dh) ** -0.5)),
        }
    _B_in = _B_setup()

    return {
        "A_x": _A_in["x"],
        "A_k_cache": _A_in["k_cache"],
        "A_v_cache": _A_in["v_cache"],
        "A_wq": _A_in["wq"],
        "A_wo": _A_in["wo"],
        "B_x": _B_in["x"],
        "B_k_cache": _B_in["k_cache"],
        "B_v_cache": _B_in["v_cache"],
        "B_wq": _B_in["wq"],
        "B_wo": _B_in["wo"],
    }

def reference(A_x, A_k_cache, A_v_cache, A_wq, A_wo, B_x, B_k_cache, B_v_cache, B_wq, B_wo):
    def _A_ref(x, k_cache, v_cache, wq, wo):
        B, Sq, D = x.shape
        Hq, Dh = 16, 256
        Hkv = k_cache.shape[1]
        rep = Hq // Hkv
        q = (lambda x, *d: x.transpose(*d))((x @ wq).reshape(B, Sq, Hq, Dh), 0, 2, 1, 3)
        k = jnp.repeat(k_cache, rep, axis=1)
        v = jnp.repeat(v_cache, rep, axis=1)
        scores = jnp.einsum("bhqd,bhkd->bhqk", q, k) * (Dh ** -0.5)
        p = _softmax(scores, axis=-1)
        o = jnp.einsum("bhqk,bhkd->bhqd", p, v)
        return (lambda x, *d: x.transpose(*d))(o, 0, 2, 1, 3).reshape(B, Sq, Hq * Dh) @ wo

    def _B_ref(x, k_cache, v_cache, wq, wo):
        B, Sq, D = x.shape
        H, Dh = 16, 256
        q = (lambda x, *d: x.transpose(*d))((x @ wq).reshape(B, Sq, H, Dh), 0, 2, 1, 3)
        scores = jnp.einsum("bhqd,bhkd->bhqk", q, k_cache) * (Dh ** -0.5)
        p = _softmax(scores, axis=-1)
        o = jnp.einsum("bhqk,bhkd->bhqd", p, v_cache)
        return (lambda x, *d: x.transpose(*d))(o, 0, 2, 1, 3).reshape(B, Sq, H * Dh) @ wo

    a = _A_ref(A_x, A_k_cache, A_v_cache, A_wq, A_wo)
    b = _B_ref(B_x, B_k_cache, B_v_cache, B_wq, B_wo)
    return jnp.concatenate([a, b], axis=-1)
```

```python
import math

import jax
import jax.numpy as jnp
from jax import lax
import jax.experimental.pallas as pl
import jax.experimental.pallas.tpu as pltpu

_NT = (((1,), (1,)), ((), ()))
_NN = (((1,), (0,)), ((), ()))
f32, bf16 = jnp.float32, jnp.bfloat16


def build(QCH=4, OCH=4, LA=2, LB=2, LO=1, LL=1, NFULL=6, MID=(8, 8), LAST=(5, 4, 3, 2, 1, 1), AB=1, dma=True, phases="12345", flags=None):
    B, SQ, D, H, HKV, SK, DH = 8, 112, 448, 16, 8, 512, 256
    T, HD = B * SQ, H * DH
    QW, OW = HD // QCH, HD // OCH
    NT_ = T // 128
    C = (DH ** -0.5) * math.log2(math.e)
    NA = B // AB
    S_Q, S_A, S_WO, S_WB, S_B, S_OUT = 0, 2, 2 + NA, 3 + NA, 4 + NA, 8 + NA
    NSEM = S_OUT + 1
    late = [(b, 0, H) for b in range(4, NFULL)]
    for b in range(max(NFULL, 4), B):
        h0 = 0
        for n in (LAST if b == B - 1 else MID):
            late.append((b, h0, n)); h0 += n
    free = list(range(0, S_WO))
    while len(free) < len(late):
        free.append(NSEM); NSEM += 1

    def softmax_pv(s, v):
        m = jnp.max(s, axis=-1, keepdims=True)
        p = jnp.exp2((s - m) * C)
        l = jnp.sum(p, axis=-1, keepdims=True)
        o = lax.dot_general(p.astype(bf16), v, _NN, preferred_element_type=f32)
        return (o * (1.0 / l)).astype(bf16)

    def kernel(xa, ka, va, wqa, woa, xb, kb, vb, wqb, wob, out,
               x_s, wq_s, woa_s, wob_s, kv_s, q_s, o_s, acc_s, out_s, sem):
        cp = pltpu.make_async_copy

        def start(cs):
            if dma:
                for mk in cs:
                    mk().start()

        def wait(cs):
            if dma:
                for mk in cs:
                    mk().wait()

        def c_wq(p, c, s):
            return lambda: cp((wqa, wqb)[p].at[:, pl.ds(c * QW, QW)], wq_s.at[p, c], sem.at[s])

        g_q0 = [lambda: cp(xa, x_s.at[0], sem.at[S_Q]), c_wq(0, 0, S_Q)]
        g_q1 = [c_wq(0, c, S_Q + 1) for c in range(1, QCH)]

        def g_a(i):
            return [(lambda j=j, b=i * AB + r: cp((ka, va)[j].at[b], kv_s.at[b // 2, j, pl.ds((b % 2) * HKV, HKV)], sem.at[S_A + i]))
                    for r in range(AB) for j in range(2)]
        g_woa = [(lambda c=c: cp(woa.at[:, pl.ds(c * OW, OW)], woa_s.at[c], sem.at[S_WO])) for c in range(OCH)]
        g_wb = ([lambda: cp(xb, x_s.at[1], sem.at[S_WB])] + [c_wq(1, c, S_WB) for c in range(QCH)]
                + [lambda: cp(wob, wob_s.at[pl.ds(64, D)], sem.at[S_WB])])

        def g_b(b, h0, n, s):
            return [(lambda j=j: cp((kb, vb)[j].at[b, pl.ds(h0, n)], kv_s.at[(b + 4) % 8, j, pl.ds(h0, n)], sem.at[s])) for j in range(2)]

        def g_out(b):
            r = pl.ds(pl.multiple_of(b * SQ, SQ), SQ)
            return [lambda: cp(out_s.at[r], out.at[r], sem.at[S_OUT])]

        start(g_q0); start(g_q1)
        for i in range(NA):
            start(g_a(i))
        start(g_woa); start(g_wb)
        for b in range(4):
            start(g_b(b, 0, H, S_B + b))

        def qchunk(p, c):
            q = lax.dot_general(x_s[p], wq_s[p, c], _NN, preferred_element_type=f32).astype(bf16)
            nh = QW // DH
            for b in range(B):
                for h in range(nh):
                    q_s[b, c * nh + h] = q[b * SQ:(b + 1) * SQ, h * DH:(h + 1) * DH]

        wob_s[0:64, :] = jnp.zeros((64, HD), bf16)
        for t in range(NT_):
            acc_s[t] = jnp.zeros((D, 128), f32)
        wait(g_q0)

        def p1(c, carry):
            if dma:
                pl.when(c == 1)(lambda: wait(g_q1))
            if "1" in phases:
                qchunk(0, c)
            return carry
        lax.fori_loop(0, QCH, p1, 0)

        def p2(it, carry):
            wait(g_a(it))
            if "2" not in phases:
                return carry
            n = AB * HKV
            ss = {}
            for g in range(n + LA):
                if g < n:
                    b, kh = it * AB + g // HKV, g % HKV
                    q = q_s[b, pl.ds(2 * kh, 2)].reshape(2 * SQ, DH)
                    ss[g] = lax.dot_general(q, kv_s[b // 2, 0, (b % 2) * HKV + kh], _NT, preferred_element_type=f32)
                if g >= LA:
                    i = g - LA
                    b, kh = it * AB + i // HKV, i % HKV
                    o = softmax_pv(ss.pop(i), kv_s[b // 2, 1, (b % 2) * HKV + kh])
                    row = pl.multiple_of(b * SQ, SQ)
                    for r in range(2):
                        col = (2 * kh + r) * DH
                        o_s[col // OW, pl.ds(row, SQ), col % OW:col % OW + DH] = o[r * SQ:(r + 1) * SQ]
            return carry
        lax.fori_loop(0, NA, p2, 0)

        for k, (b, h0, n) in enumerate(late):
            start(g_b(b, h0, n, free[k]))

        wait(g_woa)

        def p3(c, carry):
            d = lax.dot_general(woa_s[c], o_s[c], _NT, preferred_element_type=f32)
            for t in range(NT_):
                acc_s[t] += d[:, t * 128:(t + 1) * 128]
            return carry
        if "3" in phases:
            lax.fori_loop(0, OCH, p3, 0)

        wait(g_wb)
        tpi = -(-NT_ // QCH)

        def p4(c, carry):
            for u in range(tpi):
                t = jnp.minimum(c * tpi + u, NT_ - 1)
                out_s[pl.ds(pl.multiple_of(t * 128, 128), 128), 0:D] = acc_s[t].T.astype(bf16)
            qchunk(1, c)
            return carry
        if "4" in phases:
            lax.fori_loop(0, QCH, p4, 0)

        def p5(b, groups, lb, lo):
            slot = (b + 4) % 8
            ss, os_, acc = {}, {}, None
            for g in range(H + lb + lo):
                if g < H:
                    if g in groups:
                        wait(groups[g])
                    if "5" in phases:
                        ss[g] = lax.dot_general(q_s[b, g], kv_s[slot, 0, g], _NT, preferred_element_type=f32)
                if "5" not in phases:
                    continue
                i = g - lb
                if 0 <= i < H:
                    os_[i] = softmax_pv(ss.pop(i), kv_s[slot, 1, i])
                i = g - lb - lo
                if 0 <= i < H:
                    d = lax.dot_general(os_.pop(i), wob_s[:, i * DH:(i + 1) * DH], _NT, preferred_element_type=f32)
                    acc = d if acc is None else acc + d
            if "5" in phases:
                r = pl.ds(pl.multiple_of(b * SQ, SQ), SQ)
                res = acc.astype(bf16)
                out_s[r, 512:2 * D] = res[:, 128:]
                lane = lax.broadcasted_iota(jnp.int32, (SQ, 128), 1)
                out_s[r, 384:512] = jnp.where(lane < 64, out_s[r, 384:512].astype(f32), acc[:, :128]).astype(bf16)
            start(g_out(b))

        def p5_full(b, carry):
            s = jnp.where(b < 4, S_B + b, b - 4)
            p5(b, {0: g_b(b, 0, H, s)}, LB, LO)
            return carry
        lax.fori_loop(0, NFULL, p5_full, 0)
        for b in range(NFULL, B):
            p5(b, {h0: g_b(b, h0, n, free[k]) for k, (bb, h0, n) in enumerate(late) if bb == b},
               LL if b == B - 1 else LB, LO)
        if dma:
            cp(out_s, out, sem.at[S_OUT]).wait()

    def fn(A_x, A_k_cache, A_v_cache, A_wq, A_wo, B_x, B_k_cache, B_v_cache, B_wq, B_wo):
        hbm = pl.BlockSpec(memory_space=pltpu.HBM)
        return pl.pallas_call(
            kernel,
            in_specs=[hbm] * 10,
            out_specs=hbm,
            out_shape=jax.ShapeDtypeStruct((T, 2 * D), bf16),
            scratch_shapes=[
                pltpu.VMEM((2, T, D), bf16), pltpu.VMEM((2, QCH, D, QW), bf16),
                pltpu.VMEM((OCH, D, OW), bf16), pltpu.VMEM((512, HD), bf16),
                pltpu.VMEM((8, 2, H, SK, DH), bf16), pltpu.VMEM((B, H, SQ, DH), bf16),
                pltpu.VMEM((OCH, T, OW), bf16), pltpu.VMEM((NT_, D, 128), f32), pltpu.VMEM((T, 2 * D), bf16),
                pltpu.SemaphoreType.DMA((NSEM,)),
            ],
            compiler_params=pltpu.CompilerParams(vmem_limit_bytes=124 * 2**20, flags=flags),
        )(A_x.reshape(T, D), A_k_cache, A_v_cache, A_wq, A_wo.T,
          B_x.reshape(T, D), B_k_cache, B_v_cache, B_wq, B_wo.T).reshape(B, SQ, 2 * D)
    return jax.jit(fn)


_kernel = build()


@jax.jit
def pallas_concat_heads__gqa_block_cached__mha_block_cached__near_ridge_kernel(
    A_x, A_k_cache, A_v_cache, A_wq, A_wo, B_x, B_k_cache, B_v_cache, B_wq, B_wo,
):
    return _kernel(A_x, A_k_cache, A_v_cache, A_wq, A_wo, B_x, B_k_cache, B_v_cache, B_wq, B_wo)
```

```python
import contextlib
import math

import jax
import jax.numpy as jnp
from jax import lax
import jax.experimental.pallas as pl
import jax.experimental.pallas.tpu as pltpu

_NT = (((1,), (1,)), ((), ()))
_NN = (((1,), (0,)), ((), ()))
f32, bf16, u32 = jnp.float32, jnp.bfloat16, jnp.uint32


def build(QN=3, MS=4, NP=3, NK=2, NV=2, PR=64, LA=2, LB=2, LO=1, LAST=(5, 3), QPOS=(18, 18, 18, 1), OPOS=(14, 2), TP=2, WAT=0, WP=1,
          N5=2, lp=False, dma=True, prof=False, phases="12345"):
    B, SQ, D, H, HKV, SK, DH = 8, 112, 448, 16, 8, 512, 256
    T, G, NU = B * SQ, 8, 4
    NTT = T // 128
    C = (DH ** -0.5) * math.log2(math.e)
    KV_A, KV_B, WQA, WQB, WOA, WOB = 0, 128, 256, 272, 288, 304
    S_Q, S_A, S_B, S_WO, S_OUT = 0, 0, 5, 9, 10
    S_Q0, S_Q1, S_Q2, S_Q3 = 10, 11, 12, 4
    NSEM = 13
    late = [(b, 0, G) for b in range(B - 1)]
    h0 = 0
    for n in LAST:
        late.append((B - 1, h0, n)); h0 += n
    free = [0, 1, 2, 3, 4, 11, 12]
    while len(free) < len(late):
        free.append(NSEM); NSEM += 1
    last_sem = {h: free[k] for k, (b, h0, n) in enumerate(late) if b == B - 1 for h in range(h0, h0 + n)}

    def softmax_pv(s, v):
        m = jnp.max(s, axis=-1, keepdims=True)
        p = jnp.exp2(s - m)
        l = jnp.sum(p, axis=-1, keepdims=True)
        o = lax.dot_general(p.astype(bf16), v, _NN, preferred_element_type=f32)
        r = pl.reciprocal(l, approx=True)
        r = r * (2.0 - l * r)
        return (o * r).astype(bf16)

    def kernel(xa, ka, va, wqa, woa, xb, kb, vb, wqb, wob, out, x_s, pool, wob_s, qa_s, qo_s, acc_s, ini_s, out_s, sem):
        cp = pltpu.make_async_copy

        def start(cs, p=1):
            if dma:
                for mk in cs:
                    mk().start(priority=p)

        def wait(cs, name="w"):
            if dma:
                with (jax.named_scope(name) if prof else contextlib.nullcontext()):
                    for mk in cs:
                        mk().wait()

        def c_kv(src, b, h0, n, slot, r0, nr, s):
            r = pl.ds(r0, nr)
            return [lambda: cp(src.at[b, pl.ds(h0, n), r], pool.at[pl.ds(slot, n), r], sem.at[s])] if nr else []

        def c_w(src, base, h, s, r0=0):
            col = h * DH if isinstance(h, int) else pl.multiple_of(h * DH, DH)
            return [lambda: cp(src.at[:, pl.ds(col, DH)], pool.at[base + h, pl.ds(r0, D)], sem.at[s])]

        def slot(base, b, j, h):
            return base + (b * 2 + j) * G + h

        def g_kv(k, v, base, b, hs, h0, n, s, rk, rv):
            return (c_kv(k, b, hs + h0, n, slot(base, b, 0, h0), rk, SK - rk, s)
                    + c_kv(v, b, hs + h0, n, slot(base, b, 1, h0), rv, SK - rv, s))

        def pieces(src, hs, base, j, b0, nb, npc, s):
            return [c_kv(src, b0 + i // G, hs + i % G, 1, slot(base, b0 + i // G, j, i % G), k * PR, PR, s(i % G))
                    for i in range(nb * G) for k in range(npc)]

        def drip(ps, bulk=None):
            if ps:
                start(ps.pop(0), 0)
            if bulk:
                start([bulk.pop(0)], 1)

        HT = T // 2
        wq = lambda lo, hi, sm: sum([c_w(wqa, WQA, h, sm) for h in range(lo, hi)], [])
        g_q0 = [lambda: cp(xa.at[pl.ds(0, HT)], x_s.at[0, pl.ds(0, HT)], sem.at[S_Q0])] + wq(0, 2, S_Q0)
        g_q1 = [lambda: cp(xa.at[pl.ds(HT, HT)], x_s.at[0, pl.ds(HT, HT)], sem.at[S_Q1])] + wq(2, 4, S_Q1)
        g_q2 = wq(4, 8, S_Q2)
        g_q3 = wq(8, H, S_Q3)
        g_xb = [lambda: cp(xb, x_s.at[1], sem.at[S_A])]

        def g_a(u, rv=0):
            return (sum([c_w(wqb, WQB, 4 * u + i, S_A + u) for i in range(4)], [])
                    + sum([g_kv(ka, va, KV_A, 2 * u + i, 0, 0, G, S_A + u, 0, rv) for i in range(2)], []))

        def g_b(u, rv=0):
            return (sum([c_w(woa, WOA, 4 * u + i, S_B + u) for i in range(4)], [])
                    + sum([g_kv(kb, vb, KV_B, 2 * u + i, 0, 0, G, S_B + u, 0, rv) for i in range(2)], []))
        g_wob = [lambda: cp(wob, wob_s.at[pl.ds(64, D)], sem.at[S_WO])]

        start(g_q0 + g_q1 + g_q2 + g_q3 + g_xb)
        start(g_a(0, 3 * PR) + sum([c_kv(kb, i, 0, G, slot(KV_B, i, 0, 0), 0, NK * PR, S_B) for i in range(2)], []) + g_a(1))

        def qproj(p, wslot, q_s, h, r0, nr):
            q = lax.dot_general(x_s[p, r0:r0 + nr], pool[wslot, 0:D], _NN, preferred_element_type=f32)
            q = pltpu.bitcast((q * C).astype(bf16), u32)
            for c in range(2):
                q_s[2 * h + c, r0 // 2:(r0 + nr) // 2] = q[:, c * 128:(c + 1) * 128]

        def rows(b):
            return pl.ds(pl.multiple_of(b * (SQ // 2), SQ // 2), SQ // 2)

        def ld_q(q_s, b, h):
            return pltpu.bitcast(jnp.concatenate([q_s[2 * h, rows(b)], q_s[2 * h + 1, rows(b)]], axis=1), bf16)

        def st_o(b, h, o):
            o = pltpu.bitcast(o, u32)
            for c in range(2):
                qo_s[2 * H + 2 * h + c, rows(b)] = o[:, c * 128:(c + 1) * 128]

        def oproj_t(wslot, r0, h, nh, a0, ps):
            for t0, t1 in ((0, 2), (2, 4), (4, 6), (6, 7)):
                drip(ps)
                w = jnp.concatenate([pool[wslot + i, r0:r0 + D] for i in range(nh)], axis=1)
                o = jnp.concatenate([qo_s[2 * H + 2 * h + i, t0 * 64:t1 * 64] for i in range(2 * nh)], axis=1)
                d = lax.dot_general(w, pltpu.bitcast(o, bf16), _NT, preferred_element_type=f32)
                for t in range(t0, t1):
                    acc_s[t, a0:a0 + D] += d[:, (t - t0) * 128:(t - t0 + 1) * 128]

        wob_s[0:64, G * DH:] = jnp.zeros((64, G * DH), bf16)

        def zero(t, carry):
            acc_s[t] = jnp.zeros((2 * D, 128), f32)
            return carry
        lax.fori_loop(0, NTT, zero, 0)
        wait(g_q0)
        if "1" in phases:
            for h in range(2):
                qproj(0, WQA + h, qa_s, h, 0, HT)
        wait(g_q1)
        if "1" in phases:
            for h in range(2):
                qproj(0, WQA + h, qa_s, h, HT, HT)
        for h in range(2, 4):
            start(g_a(h))
            if "1" in phases:
                qproj(0, WQA + h, qa_s, h, 0, T)
        wait(g_q2)

        def p1(c, carry):
            if dma:
                pl.when(c == 1)(lambda: wait(g_q3))
            ps = [c_kv(va, i // G, i % G, 1, slot(KV_A, i // G, 1, i % G), c * PR, PR, S_A) for i in range(2 * G)]
            for i in range(4):
                for m in range(MS):
                    drip(ps)
                    if "1" in phases:
                        qproj(0, WQA + 4 + 4 * c + i, qa_s, 4 + 4 * c + i, m * T // MS, T // MS)
            while ps:
                drip(ps)
            return carry
        lax.fori_loop(0, 3, p1, 0)
        wait(g_xb)

        def p2(u, carry):
            wait(g_a(u))
            bulk = (sum([c_w(woa, WOA, 4 * u + i, S_B + u) for i in range(4)], [])
                    + c_kv(kb, 2 * u, 0, G, slot(KV_B, 2 * u, 0, 0), NK * PR, SK - NK * PR, S_B + u)
                    + c_kv(kb, 2 * u + 1, 0, G, slot(KV_B, 2 * u + 1, 0, 0), NK * PR, SK - NK * PR, S_B + u)
                    + c_kv(vb, 2 * u, 0, G, slot(KV_B, 2 * u, 1, 0), NP * PR, SK - NP * PR, S_B + u)
                    + c_kv(vb, 2 * u + 1, 0, G, slot(KV_B, 2 * u + 1, 1, 0), NP * PR, SK - NP * PR, S_B + u))
            ps = pieces(vb, 0, KV_B, 1, 2 * u, 2, NP, lambda h: S_B + u)
            n, ss = 2 * G, {}
            for g in range(n + LA):
                if g < n:
                    drip(ps)
                    if "2" in phases:
                        b, kh = 2 * u + g // G, g % G
                        q = jnp.concatenate([ld_q(qa_s, b, 2 * kh + r) for r in range(2)], axis=0)
                        ss[g] = lax.dot_general(q, pool[slot(KV_A, b, 0, kh)], _NT, preferred_element_type=f32)
                for i, pos in enumerate(QPOS):
                    if g == n + LA - pos:
                        for m in range(MS):
                            drip(ps, bulk)
                            if "2" in phases:
                                qproj(1, WQB + 4 * u + i, qo_s, 4 * u + i, m * T // MS, T // MS)
                i = g - LA
                if i >= 0:
                    drip(ps)
                    if "2" in phases:
                        b, kh = 2 * u + i // G, i % G
                        o = softmax_pv(ss.pop(i), pool[slot(KV_A, b, 1, kh)])
                        for r in range(2):
                            st_o(b, 2 * kh + r, o[r * SQ:(r + 1) * SQ])
            while ps or bulk:
                drip(ps, bulk)
            return carry
        lax.fori_loop(0, NU, p2, 0)

        start(g_wob)

        def late_sem(b, h):
            s = last_sem[h]
            for k in range(B - 1):
                s = jnp.where(b == k, free[k], s)
            return s

        def p3(u, carry):
            wait(g_b(u))
            bulk = g_kv(kb, vb, KV_A, 2 * u, G, 0, G, late_sem(2 * u, 0), NK * PR, NV * PR)
            for bb, h0, n in late[B - 1:]:
                bulk += g_kv(kb, vb, KV_A, 2 * u + 1, G, h0, n, late_sem(2 * u + 1, h0), NK * PR, NV * PR)
            nxt = u < NU - 1
            ps = []
            for i in range(2):
                sm = jnp.where(nxt, S_B + u + 1, free[i])
                ps += pieces(kb, jnp.where(nxt, 0, G), jnp.where(nxt, KV_B, KV_A), 0, jnp.where(nxt, 2 * u + 2 + i, i), 1, NK, lambda h: sm)
            n, ss = 2 * G, {}
            for g in range(n + LB):
                if g < n:
                    drip(ps, bulk)
                    if "3" in phases:
                        b, h = 2 * u + g // G, g % G
                        ss[g] = lax.dot_general(ld_q(qo_s, b, h), pool[slot(KV_B, b, 0, h)], _NT, preferred_element_type=f32)
                for i, pos in enumerate(OPOS):
                    if g == n + LB - pos and "3" in phases:
                        nh = 4 // len(OPOS)
                        oproj_t(WOA + 4 * u + i * nh, 0, 4 * u + i * nh, nh, 0, ps)
                i = g - LB
                if i >= 0:
                    drip(ps)
                    if "3" in phases:
                        b, h = 2 * u + i // G, i % G
                        o = pltpu.bitcast(softmax_pv(ss.pop(i), pool[slot(KV_B, b, 1, h)]), u32)
                        for c in range(2):
                            qa_s[2 * h + c, rows(b)] = o[:, c * 128:(c + 1) * 128]
            while ps:
                drip(ps)
            return carry
        lax.fori_loop(0, NU, p3, 0)

        for k, (b, h0, n) in enumerate(late):
            if b >= 2:
                start(c_kv(kb, b, G + h0, n, slot(KV_A, b, 0, h0), 0, NK * PR, free[k]), 0)
        wait(g_wob)

        def p4(c, carry):
            nh = G // N5
            h = c * nh
            ps = [c_kv(vb, 0, G + h, nh, slot(KV_A, 0, 1, h), k * PR, PR, free[0]) for k in range(NV)]
            for t in range(NTT):
                drip(ps)
                if "4" in phases:
                    w = wob_s[64:64 + D, pl.ds(pl.multiple_of(h * DH, nh * DH), nh * DH)]
                    o = jnp.concatenate([qa_s[2 * h + i, t * 64:(t + 1) * 64] for i in range(2 * nh)], axis=1)
                    acc_s[t, D:2 * D] += lax.dot_general(w, pltpu.bitcast(o, bf16), _NT, preferred_element_type=f32)
            while ps:
                drip(ps)
            return carry
        lax.fori_loop(0, N5, p4, 0)

        def p5(b, groups, ps, tr):
            ss, os_, acc = {}, {}, None
            for g in range(G + LB + LO):
                if g < G:
                    if g in groups:
                        wait(groups[g])
                        if not tr and g == WAT:
                            start(early, WP)
                    drip(ps)
                    if "5" in phases:
                        ss[g] = lax.dot_general(ld_q(qo_s, b, G + g), pool[slot(KV_A, b, 0, g)], _NT, preferred_element_type=f32)
                if tr and g == TP and "5" in phases:
                    r = pl.ds(pl.multiple_of(b * 128, 128), 128)
                    a = acc_s[b].T
                    out_s[r, 0:384] = a[:, 0:384].astype(bf16)
                    ini_s[r] = a[:, 384:]
                i = g - LB
                if 0 <= i < G:
                    drip(ps)
                    if "5" in phases:
                        os_[i] = softmax_pv(ss.pop(i), pool[slot(KV_A, b, 1, i)])
                i = g - LB - LO
                if 0 <= i < G:
                    drip(ps)
                    if "5" in phases:
                        d = lax.dot_general(os_.pop(i), wob_s[:, (G + i) * DH:(G + i + 1) * DH], _NT, preferred_element_type=f32)
                        acc = d if acc is None else acc + d
            while ps:
                drip(ps)
            r = pl.ds(pl.multiple_of(b * SQ, SQ), SQ)
            if "5" in phases:
                ini = ini_s[r]
                res = ini + acc
                lane = lax.broadcasted_iota(jnp.int32, (SQ, 128), 1)
                out_s[r, 384:512] = jnp.where(lane < 64, ini[:, :128], res[:, :128]).astype(bf16)
                out_s[r, 512:2 * D] = res[:, 128:].astype(bf16)
            return r

        def p5_loop(b, carry):
            sl = {h: late_sem(b + 1, h) for h in range(G)}
            r = p5(b, {0: g_kv(kb, vb, KV_A, b, G, 0, G, late_sem(b, 0), 0, 0)},
                   pieces(vb, G, KV_A, 1, b + 1, 1, NV, lambda h: sl[h]), True)
            return carry
        lax.fori_loop(0, B - 1, p5_loop, 0)
        rl = pl.ds((B - 1) * SQ, SQ)
        rf = pl.ds(0, (B - 1) * SQ)
        early = [lambda: cp(out_s.at[rf], out.at[rf], sem.at[S_OUT]),
                 lambda: cp(out_s.at[rl, pl.ds(0, 384)], out.at[rl, pl.ds(0, 384)], sem.at[S_OUT])]
        p5(B - 1, {h0: g_kv(kb, vb, KV_A, b, G, h0, n, free[k], 0, 0) for k, (b, h0, n) in enumerate(late) if b == B - 1}, [], False)
        start([lambda: cp(out_s.at[rl, pl.ds(384, 512)], out.at[rl, pl.ds(384, 512)], sem.at[S_OUT])], 0)
        wait([lambda: cp(out_s, out, sem.at[S_OUT])])

    def fn(A_x, A_k_cache, A_v_cache, A_wq, A_wo, B_x, B_k_cache, B_v_cache, B_wq, B_wo):
        hbm = pl.BlockSpec(memory_space=pltpu.HBM)
        return pl.pallas_call(
            kernel,
            in_specs=[hbm] * 10,
            out_specs=hbm,
            out_shape=jax.ShapeDtypeStruct((T, 2 * D), bf16),
            scratch_shapes=[
                pltpu.VMEM((2, T, D), bf16), pltpu.VMEM((304, SK, DH), bf16), pltpu.VMEM((512, H * DH), bf16),
                pltpu.VMEM((2 * H, T // 2, 128), u32), pltpu.VMEM((4 * H, T // 2, 128), u32),
                pltpu.VMEM((NTT, 2 * D, 128), f32), pltpu.VMEM((T, 512), f32), pltpu.VMEM((T, 2 * D), bf16),
                pltpu.SemaphoreType.DMA((NSEM,)),
            ],
            compiler_params=pltpu.CompilerParams(
                vmem_limit_bytes=126 * 2**20, disable_bounds_checks=True,
                flags={'XLA_TPU_FORCE_LP_LLO_SCHEDULER': True} if lp else None),
        )(A_x.reshape(T, D), A_k_cache, A_v_cache, A_wq, A_wo.T,
          B_x.reshape(T, D), B_k_cache, B_v_cache, B_wq, B_wo.T).reshape(B, SQ, 2 * D)
    return jax.jit(fn)


_kernel = build(LAST=(8,))


@jax.jit
def pallas_concat_heads__gqa_block_cached__mha_block_cached__near_ridge_kernel(
    A_x, A_k_cache, A_v_cache, A_wq, A_wo, B_x, B_k_cache, B_v_cache, B_wq, B_wo,
):
    return _kernel(A_x, A_k_cache, A_v_cache, A_wq, A_wo, B_x, B_k_cache, B_v_cache, B_wq, B_wo)
```

```python
import contextlib
import functools
import math

import jax
import jax.numpy as jnp
from jax import lax
import jax.experimental.pallas as pl
import jax.experimental.pallas.tpu as pltpu

_NT = (((1,), (1,)), ((), ()))
_NN = (((1,), (0,)), ((), ()))
f32, bf16, u32 = jnp.float32, jnp.bfloat16, jnp.uint32


def build(QN=2, MS=3, NP=3, NK=3, NV=4, PR=64, LA=1, LB=1, LC=2, LO=1, N5=1, P0=(1, 1), TP=2, PRED=True, WP=1, PRE3=False, F0=((224, 1), (448, 1), (448, 2), (896, 2), (896, 4)), LG=2, HALF=2, HK=1, HV=2, N1=2, NX=3, EW=2, XS=False, HK3=1, HV3=2, HK5=1, HV5=2, F4=6, PRE5=True, lp=False,
          dma=True, prof=False, phases="12345"):
    B, SQ, D, H, HKV, SK, DH = 8, 112, 448, 16, 8, 512, 256
    T = B * SQ
    NA, NB = 4, 5
    HT = 2 * NB
    HL = H - HT
    NTT = T // 128
    MB = {2: (0, 448, 896), 3: (0, 304, 608, 896), 4: (0, 224, 448, 672, 896)}[MS]
    C = (DH ** -0.5) * math.log2(math.e)
    KV_A, KV_B, WQA, WQB = 0, 128, 288, 304
    S_A, S_B, S_WO, S_OUT = 0, 8, 13, 12
    S_Q0, S_Q1, S_Q2, S_Q3 = 4, 5, 6, 7
    NSEM = 14

    def softmax_pv(s, v, pre=True):
        m = jnp.max(s, axis=-1, keepdims=True)
        p = jnp.exp2(s - m)
        l = jnp.sum(p, axis=-1, keepdims=True)
        r = pl.reciprocal(l, approx=True)
        r = r * (2.0 - l * r)
        if pre:
            return lax.dot_general((p * r).astype(bf16), v, _NN, preferred_element_type=f32).astype(bf16)
        return (lax.dot_general(p.astype(bf16), v, _NN, preferred_element_type=f32) * r).astype(bf16)

    def kernel(xa, ka, va, wqa, woa, xb, kb, vb, wqb, wob, out,
               x_s, pool, wo_s, qa_s, qb_s, o_s, acc_s, out_s, sem):
        cp = pltpu.make_async_copy

        def start(cs, p=1):
            if dma:
                for mk in cs:
                    mk().start(priority=p)

        def wait(cs, name="w"):
            if dma:
                with (jax.named_scope(name) if prof and name else contextlib.nullcontext()):
                    for mk in cs:
                        mk().wait()

        def drip(ps, bulk=None):
            if ps:
                mk = ps.pop(0)
                if isinstance(mk, tuple):
                    pl.when(mk[0])(functools.partial(start, [mk[1]], 0))
                else:
                    start([mk], 0)
            if bulk:
                start([bulk.pop(0)], 1)

        def c_kv(src, b, h, slot, r0, nr, s):
            r = pl.ds(r0, nr)
            n = b.size if isinstance(b, pl.Slice) else h.size
            return lambda: cp(src.at[b, h, r], pool.at[pl.ds(slot, n), r], sem.at[s])

        def pieces(src, tiles, npc):
            return [c_kv(src, b, pl.ds(h, 1), sl, k * PR, PR, s) for b, h, sl, s in tiles for k in range(npc)]

        def c_wq(src, base, h, s):
            col = h * DH if isinstance(h, int) else pl.multiple_of(h * DH, DH)
            return lambda: cp(src.at[:, pl.ds(col, DH)], pool.at[base + h, pl.ds(0, D)], sem.at[s])

        a_slot = lambda b, j, h: KV_A + (b * 2 + j) * HKV + h
        t_slot = lambda b, j, h: KV_B + (h * 2 + j) * B + b
        l_slot = lambda b, j, h: KV_A + (b * 2 + j) * HL + h - HT

        def g_a(u, rv=0):
            cs = [c_wq(wqb, WQB, 4 * u + i, S_A + u) for i in range(4)]
            for b in (2 * u, 2 * u + 1):
                cs += [c_kv(ka, b, pl.ds(0, HKV), a_slot(b, 0, 0), 0, SK, S_A + u),
                       c_kv(va, b, pl.ds(0, HKV), a_slot(b, 1, 0), rv, SK - rv, S_A + u)]
            return cs

        def g_t(u, rk=0, rv=0):
            return [c_kv(src, pl.ds(0, B), 2 * u + i, t_slot(0, j, 2 * u + i), r0, SK - r0, S_B + u)
                    for i in range(2) for j, (src, r0) in enumerate(((kb, rk), (vb, rv)))]

        def c_wo(src, c_src, c_dst, nc, s):
            return lambda: cp(src.at[:, pl.ds(c_src, nc)], wo_s.at[:, pl.ds(c_dst, nc)], sem.at[s])

        def c_woa(u):
            col = pl.multiple_of(u * 4 * DH, 4 * DH)
            return c_wo(woa, col, col, 4 * DH, S_B + u)

        wq = lambda lo, hi, s: [c_wq(wqa, WQA, h, s) for h in range(lo, hi)]
        steps, (rp, hp) = [], (0, 0)
        for k, (r, h) in enumerate(F0):
            sm = (4, 5, 9, 10, 11, 12, 13)[k]
            cs = [functools.partial(cp, xa.at[pl.ds(rp, r - rp)], x_s.at[0, pl.ds(rp, r - rp)], sem.at[sm])] if r > rp else []
            steps.append((cs + wq(hp, h, sm), [(i, rp, r - rp) for i in range(hp) if r > rp] + [(i, 0, r) for i in range(hp, h)]))
            rp, hp = r, h
        HP = (H - 4) // QN
        g_q2, g_q3 = wq(4, 4 + HP, S_Q2), wq(4 + HP, H, S_Q3)
        g_xb = [functools.partial(cp, xb.at[:, pl.ds(c0, nc)], x_s.at[1, :, pl.ds(c0, nc)], sem.at[S_A])
                for c0, nc in (((0, 384), (384, 64)) if XS else ((0, D),))]
        g_wob = [c_wo(wob, 4 * DH, (H + 4) * DH, (H - 4) * DH, S_WO)]

        start(sum([cs for cs, _ in steps], []) + g_q2 + g_q3 + g_xb + g_a(0, QN * N1 * PR)
              + g_a(1, NX * PR))

        def ld_kv(slot, ps, mode):
            if mode == 0:
                return pool[slot]
            if mode == 2:
                lo = pool[slot, :, 0:128]
                drip(ps)
                return jnp.concatenate([lo, pool[slot, :, 128:DH]], axis=1)
            lo = pool[slot, 0:SK // 2]
            drip(ps)
            return jnp.concatenate([lo, pool[slot, SK // 2:SK]], axis=0)

        def qproj(p, wslot, q_s, h, r0, nr, ps=None):
            if ps is not None and HALF & 2:
                lo = pool[wslot, 0:D, 0:128]
                drip(ps)
                w = jnp.concatenate([lo, pool[wslot, 0:D, 128:DH]], axis=1)
            else:
                w = pool[wslot, 0:D]
            q = lax.dot_general(x_s[p, r0:r0 + nr], w, _NN, preferred_element_type=f32)
            q = pltpu.bitcast((q * C).astype(bf16), u32)
            for c in range(2):
                q_s[2 * h + c, r0 // 2:(r0 + nr) // 2] = q[:, c * 128:(c + 1) * 128]

        def rows(b):
            return pl.ds(pl.multiple_of(b * (SQ // 2), SQ // 2), SQ // 2)

        def ld_q(q_s, b, h):
            return pltpu.bitcast(jnp.concatenate([q_s[2 * h, rows(b)], q_s[2 * h + 1, rows(b)]], axis=1), bf16)

        def st_o(b, h, o):
            o = pltpu.bitcast(o, u32)
            for c in range(2):
                o_s[2 * h + c, rows(b)] = o[:, c * 128:(c + 1) * 128]
        def zero(t, carry):
            acc_s[t] = jnp.zeros((2 * D, 128), f32)
            return carry
        lax.fori_loop(0, NTT, zero, 0)
        for k, (cs, work) in enumerate(steps):
            wait(cs, k == 0 and "w")
            if k == len(steps) - 1:
                start(g_a(2, NX * PR))
            for h, r0, nr in work:
                qproj(0, WQA + h, qa_s, h, r0, nr)
        wait(g_q2)

        def p1(c, carry):
            if dma:
                pl.when(c == 1)(lambda: (start(g_a(3, NX * PR) + [c_kv(kb, pl.ds(0, B), i, t_slot(0, 0, i), 0, NK * PR, S_B) for i in range(2)]), wait(g_q3))[1])
            ps = [c_kv(va, b, pl.ds(h, 1), a_slot(b, 1, h), (c * N1 + k) * PR, PR, S_A)
                  for b in range(2) for h in range(HKV) for k in range(N1)]
            for i in range(HP):
                for m in range(MS):
                    if "1" in phases:
                        qproj(0, WQA + 4 + HP * c + i, qa_s, 4 + HP * c + i, MB[m], MB[m + 1] - MB[m], ps)
                    drip(ps)
                    if len(ps) > N1 * (HP * MS - (i * MS + m) - 2):
                        drip(ps)
            while ps:
                drip(ps)
            return carry
        lax.fori_loop(0, QN, p1, 0)
        wait(g_xb)

        def p2(u, carry):
            wait(g_a(u))
            bulk = [c_woa(u)] + g_t(u, NK * PR, NP * PR)
            ps = pieces(vb, [(b, 2 * u + i, t_slot(b, 1, 2 * u + i), S_B + u) for i in range(2) for b in range(B)], NP)
            un = jnp.minimum(u + 1, NA - 1)
            ps = [(u < NA - 1, mk) for mk in pieces(va, [(2 * un + i, h, a_slot(2 * un + i, 1, h), S_A + un)
                                                         for i in range(2) for h in range(HKV)], NX)] + ps
            n, ss = 2 * HKV, {}
            for g in range(n + LA):
                if g < n:
                    drip(ps)
                    if "2" in phases:
                        b, kh = 2 * u + g // HKV, g % HKV
                        q = jnp.concatenate([ld_q(qa_s, b, 2 * kh + r) for r in range(2)], axis=0)
                        ss[g] = lax.dot_general(q, ld_kv(a_slot(b, 0, kh), ps, HK), _NT, preferred_element_type=f32)
                i = g - LA
                if i >= 0:
                    drip(ps, bulk)
                    if "2" in phases:
                        qproj(1, WQB + 4 * u + i // 4, qb_s, 4 * u + i // 4, (i % 4) * T // 4, T // 4, ps)
                    drip(ps)
                    if "2" in phases:
                        b, kh = 2 * u + i // HKV, i % HKV
                        o = softmax_pv(ss.pop(i), ld_kv(a_slot(b, 1, kh), ps, HV))
                        for r in range(2):
                            st_o(b, 2 * kh + r, o[r * SQ:(r + 1) * SQ])
            return carry
        lax.fori_loop(0, NA, p2, 0)

        start([c_wo(wob, 0, H * DH, 4 * DH, S_B + NA)] + g_t(NA, NK * PR, 0) + g_wob
              + [c_kv(vb, b, pl.ds(HT, HL), l_slot(b, 1, HT), 0, NV * PR, b) for b in range(1)])

        def oproj_t(h, nh, a0, t0, t1):
            w = wo_s[:, pl.ds(h * DH if isinstance(h, int) else pl.multiple_of(h * DH, DH), nh * DH)]
            o = jnp.concatenate([o_s[2 * h + i, t0 * 64:t1 * 64] for i in range(2 * nh)], axis=1)
            d = lax.dot_general(w, pltpu.bitcast(o, bf16), _NT, preferred_element_type=f32)
            for t in range(t0, t1):
                acc_s[t, pl.ds(a0, D)] += d[:, (t - t0) * 128:(t - t0 + 1) * 128]

        def late(b, h2, s):
            return [c_kv(kb, b, pl.ds(HT, 2), l_slot(b, 0, HT), NK * PR, SK - NK * PR, s),
                    c_kv(kb, b, pl.ds(HT + 2, h2 - HT - 2), l_slot(b, 0, HT + 2), 0, SK, s),
                    c_kv(vb, b, pl.ds(HT, h2 - HT), l_slot(b, 1, HT), NV * PR, SK - NV * PR, s)]

        def p3(u, carry):
            wait([c_woa(0 * u)][:0] + [lambda: cp(wo_s.at[:, pl.ds(0, 4 * DH)], wo_s.at[:, pl.ds(0, 4 * DH)], sem.at[S_B + u])] + g_t(u))
            if dma:
                pl.when(u > 1)(lambda: start(late(2 * u - 4, H, 2 * u - 4) + late(2 * u - 3, H, 2 * u - 3)))
            nxt = u < NB - 1
            ps = pieces(kb, [(b, 2 * u + 2 + i, jnp.where(nxt, t_slot(b, 0, 2 * u + 2 + i), l_slot(b, 0, HT + i)),
                              jnp.where(nxt, S_B + u + 1, b)) for i in range(2) for b in range(B)], NK)
            a0 = pl.multiple_of(jnp.where(u < NA, 0, D), D)
            n, ss, pend = 2 * B, {}, None
            for g in range(n + LB):
                if g < n:
                    if "3" in phases:
                        b, h = g % B, 2 * u + g // B
                        ss[g] = lax.dot_general(ld_q(qb_s, b, h), ld_kv(t_slot(b, 0, h), ps if g else [], HK3), _NT, preferred_element_type=f32)
                    if g > 0:
                        drip(ps)
                    if 0 < g < 5 and not HK3:
                        drip(ps)
                k = n + LB - 1 - g
                if k % 2 == 0 and k // 2 < NTT and "3" in phases:
                    t = NTT - 1 - k // 2
                    oproj_t(4 * u, 4, a0, t, t + 1)
                i = g - LB
                if i >= 0:
                    drip(ps)
                    if "3" in phases:
                        if pend:
                            st_o(*pend)
                        b, h = i % B, 2 * u + i // B
                        pend = (b, H + h, softmax_pv(ss.pop(i), ld_kv(t_slot(b, 1, h), ps, HV3), PRE3))
            if pend:
                st_o(*pend)
            return carry
        lax.fori_loop(0, NB, p3, 0)

        def g_l(b, h0, n, s):
            return [c_kv(src, b, pl.ds(h0, n), l_slot(b, j, h0), 0, SK, s) for j, src in enumerate((kb, vb))]

        def c_out(r0, nr, c0, nc):
            r, c = pl.ds(r0, nr), pl.ds(c0, nc)
            return [lambda: cp(out_s.at[r, c], out.at[r, c], sem.at[S_OUT])]

        def emit(t, c0, c1):
            out_s[pl.ds(t * 128 if isinstance(t, int) else pl.multiple_of(t * 128, 128), 128), c0:c1] = acc_s[t, c0:c1].T.astype(bf16)

        h2 = H - LG
        wait(g_wob)
        for b in range(B - 2, B):
            s2 = S_B + 2 * (b - (B - 2))
            start(late(b, h2, b) + [c_kv(kb, b, pl.ds(h2, LG), l_slot(b, 0, h2), 0, SK, s2),
                                    c_kv(vb, b, pl.ds(h2, LG), l_slot(b, 1, h2), NV * PR, SK - NV * PR, s2 + 1)])
        emit(NTT - 1, 0, 384)
        oproj_t(H + 4, HT - 4, D, 0, NTT - 1)

        def p5(b, carry):
            split = b >= B - 2
            s2 = S_B + 2 * jnp.maximum(b - (B - 2), 0)
            wait(g_l(b, HT, HL - LG, b))
            pl.when(jnp.logical_not(split))(lambda: wait(g_l(b, h2, LG, b), None))
            early = lambda: start(c_out(0, T - 256, 0, 2 * D) + c_out(T - 128, 128, 0, 384), WP)
            if EW == 0:
                pl.when(b == B - 1)(early)
            nb = jnp.minimum(b + 1, B - 1)
            vs = jnp.where(nb >= B - 2, S_B + 2 * (nb - (B - 2)) + 1, nb)
            ps = pieces(vb, [(nb, h, l_slot(nb, 1, h), vs if h >= h2 else nb) for h in range(HT, H)], NV)

            ps = [(b < B - 1, mk) for mk in ps]
            t = jnp.where(b == 0, NTT - 1, b - 1)
            hb = jnp.where(b == 0, H + 4, H + HT)
            ss, pend, acc = {}, None, None
            for g in range(HL + LC + 2):
                if g < HL:
                    if g == HL - LG:
                        pl.when(split)(lambda: wait(g_l(b, h2, LG, s2)[:1], None))
                        if EW == 2:
                            pl.when(b == B - 1)(early)
                    ss[g] = lax.dot_general(ld_q(qb_s, b, HT + g), ld_kv(l_slot(b, 0, HT + g), ps if g else [], HK5), _NT, preferred_element_type=f32)
                    if g > 0:
                        drip(ps)
                        if not HK5 or g < 3:
                            drip(ps)
                if g == TP:
                    emit(jnp.maximum(b - 2, 0), 0, 2 * D)
                if g == HL + LC + 1:
                    st_o(*pend)
                k = g - (HL + LC - 1)
                if k >= 0:
                    h = hb + 2 * k
                    o = jnp.concatenate([o_s[2 * h + j, pl.ds(pl.multiple_of(t * 64, 64), 64)] for j in range(4)], axis=1)
                    d = lax.dot_general(wo_s[:, pl.ds(pl.multiple_of(h * DH, 2 * DH), 2 * DH)], pltpu.bitcast(o, bf16), _NT,
                                        preferred_element_type=f32)
                    acc = d if acc is None else acc + d
                i = g - LC
                if 0 <= i < HL:
                    if pend:
                        st_o(*pend)
                    if i == HL - LG:
                        pl.when(split)(lambda: wait(g_l(b, h2, LG, s2 + 1)[1:], None))
                        if EW == 1:
                            pl.when(b == B - 1)(early)
                    pend = (b, H + HT + i, softmax_pv(ss.pop(i), ld_kv(l_slot(b, 1, HT + i), ps, HV5), PRE5))
                    drip(ps)
            assert not ps
            acc_s[t, D:2 * D] += acc
            return carry
        lax.fori_loop(0, B, p5, 0)
        start(c_out(T - 256, 128, 0, 2 * D), 0)
        emit(NTT - 1, 384, 2 * D)
        start(c_out(T - 128, 128, 384, 512), 0)
        wait(c_out(0, T, 0, 2 * D))

    def fn(A_x, A_k_cache, A_v_cache, A_wq, A_wo, B_x, B_k_cache, B_v_cache, B_wq, B_wo):
        hbm = pl.BlockSpec(memory_space=pltpu.HBM)
        return pl.pallas_call(
            kernel,
            in_specs=[hbm] * 10,
            out_specs=hbm,
            out_shape=jax.ShapeDtypeStruct((T, 2 * D), bf16),
            scratch_shapes=[
                pltpu.VMEM((2, T, D), bf16), pltpu.VMEM((320, SK, DH), bf16),
                pltpu.VMEM((D, 2 * H * DH), bf16),
                pltpu.VMEM((2 * H, T // 2, 128), u32), pltpu.VMEM((2 * H, T // 2, 128), u32),
                pltpu.VMEM((4 * H, T // 2, 128), u32),
                pltpu.VMEM((NTT, 2 * D, 128), f32), pltpu.VMEM((T, 2 * D), bf16),
                pltpu.SemaphoreType.DMA((NSEM,)),
            ],
            compiler_params=pltpu.CompilerParams(
                vmem_limit_bytes=127 * 2**20, disable_bounds_checks=True,
                flags={'XLA_TPU_FORCE_LP_LLO_SCHEDULER': True} if lp else None),
        )(A_x.reshape(T, D), A_k_cache, A_v_cache, A_wq, A_wo.T,
          B_x.reshape(T, D), B_k_cache, B_v_cache, B_wq, B_wo.T).reshape(B, SQ, 2 * D)
    return jax.jit(fn)


_kernel = build()


@jax.jit
def pallas_concat_heads__gqa_block_cached__mha_block_cached__near_ridge_kernel(
    A_x, A_k_cache, A_v_cache, A_wq, A_wo, B_x, B_k_cache, B_v_cache, B_wq, B_wo,
):
    return _kernel(A_x, A_k_cache, A_v_cache, A_wq, A_wo, B_x, B_k_cache, B_v_cache, B_wq, B_wo)
```

```python
import functools
import math

import jax
import jax.numpy as jnp
from jax import lax
import jax.experimental.pallas as pl
import jax.experimental.pallas.tpu as pltpu

_NT = (((1,), (1,)), ((), ()))
_NN = (((1,), (0,)), ((), ()))

B, SQ, D, H, HKV, SK, DH = 8, 112, 448, 16, 8, 512, 256
T = B * SQ
NTT = T // 128
NA, NB = 4, 5
HT = 2 * NB
HL = H - HT
LG = 2
SCALE = (DH ** -0.5) * math.log2(math.e)

KV_A, KV_B, WQA, WQB, NSLOT = 0, 2 * B * HKV, 2 * B * (HKV + HT), 2 * B * (HKV + HT) + H, 2 * B * (HKV + HT) + 2 * H
S_A, S_Q2, S_Q3, S_B, S_OUT, S_WO, NSEM = 0, 6, 7, 8, 12, 13, 14
S_FIRST = (4, 5, 9, 10, 11, 12, 13)
FIRST = ((224, 1), (448, 1), (448, 2), (672, 2), (896, 2), (896, 3), (896, 4))
QN = 2
MB = (0, 304, 608, 896)
PR = 64
N1, NX, NP, NK, NV = 2, 3, 3, 3, 3


def _pv(s, v, normalize_first):
    p = jnp.exp2(s - jnp.max(s, axis=-1, keepdims=True))
    l = jnp.sum(p, axis=-1, keepdims=True)
    r = pl.reciprocal(l, approx=True)
    r = r * (2.0 - l * r)
    if normalize_first:
        o = lax.dot_general((p * r).astype(v.dtype), v, _NN, preferred_element_type=jnp.float32)
    else:
        o = lax.dot_general(p.astype(v.dtype), v, _NN, preferred_element_type=jnp.float32) * r
    return o.astype(v.dtype)


def _mult(i, n):
    return i if isinstance(i, int) else pl.multiple_of(i, n)


def _kernel(xa, ka, va, wqa, woa, xb, kb, vb, wqb, wob, out,
            x_s, pool, wo_s, qa_s, qb_s, o_s, acc_s, out_s, sem):
    f32, bf16, u32 = jnp.float32, jnp.bfloat16, jnp.uint32

    def copy(src, dst, s):
        return lambda: pltpu.make_async_copy(src, dst, sem.at[s])

    def start(cs, priority=1):
        for c in cs:
            c().start(priority=priority)

    def wait(cs):
        for c in cs:
            c().wait()

    def drip(ps):
        if ps:
            cond, c = ps.pop(0)
            if cond is None:
                start([c], 0)
            else:
                pl.when(cond)(functools.partial(start, [c], 0))

    def c_kv(src, b, h, slot, r0, nr, s):
        n = b.size if isinstance(b, pl.Slice) else h.size
        return copy(src.at[b, h, pl.ds(r0, nr)], pool.at[pl.ds(slot, n), pl.ds(r0, nr)], s)

    def pieces(src, tiles, n, cond=None, k0=0):
        return [(cond, c_kv(src, b, pl.ds(h, 1), slot, (k0 + k) * PR, PR, s))
                for b, h, slot, s in tiles for k in range(n)]

    def c_wq(src, base, h, s):
        return copy(src.at[:, pl.ds(_mult(h * DH, DH), DH)], pool.at[base + h, pl.ds(0, D)], s)

    def c_wo(src, h_src, h_dst, n, s):
        return copy(src.at[:, pl.ds(_mult(h_src * DH, DH), n * DH)], wo_s.at[:, pl.ds(_mult(h_dst * DH, DH), n * DH)], s)

    def c_out(r0, nr, c0, nc):
        return [copy(out_s.at[pl.ds(r0, nr), pl.ds(c0, nc)], out.at[pl.ds(r0, nr), pl.ds(c0, nc)], S_OUT)]

    a_slot = lambda b, j, h: KV_A + (b * 2 + j) * HKV + h
    t_slot = lambda b, j, h: KV_B + (h * 2 + j) * B + b
    l_slot = lambda b, j, h: KV_A + (b * 2 + j) * HL + h - HT

    def g_a(u, rv=0):
        cs = [c_wq(wqb, WQB, 4 * u + i, S_A + u) for i in range(4)]
        for b in (2 * u, 2 * u + 1):
            cs += [c_kv(ka, b, pl.ds(0, HKV), a_slot(b, 0, 0), 0, SK, S_A + u),
                   c_kv(va, b, pl.ds(0, HKV), a_slot(b, 1, 0), rv, SK - rv, S_A + u)]
        return cs

    def g_t(u, rk=0, rv=0):
        return [c_kv(src, pl.ds(0, B), 2 * u + i, t_slot(0, j, 2 * u + i), r0, SK - r0, S_B + u)
                for i in range(2) for j, (src, r0) in enumerate(((kb, rk), (vb, rv)))]

    def g_l(b, h0, n, s):
        return [c_kv(src, b, pl.ds(h0, n), l_slot(b, j, h0), 0, SK, s) for j, src in enumerate((kb, vb))]

    def late(b, h1, s):
        return [c_kv(kb, b, pl.ds(HT, 2), l_slot(b, 0, HT), NK * PR, SK - NK * PR, s),
                c_kv(kb, b, pl.ds(HT + 2, h1 - HT - 2), l_slot(b, 0, HT + 2), 0, SK, s),
                c_kv(vb, b, pl.ds(HT, h1 - HT), l_slot(b, 1, HT), NV * PR, SK - NV * PR, s)]

    def ld_k(slot, ps):
        lo = pool[slot, 0:SK // 2]
        drip(ps)
        return jnp.concatenate([lo, pool[slot, SK // 2:SK]], axis=0)

    def ld_cols(slot, nr, ps):
        lo = pool[slot, 0:nr, 0:128]
        drip(ps)
        return jnp.concatenate([lo, pool[slot, 0:nr, 128:DH]], axis=1)

    def qproj(p, slot, q_s, h, r0, nr, ps=None):
        w = pool[slot, 0:D] if ps is None else ld_cols(slot, D, ps)
        q = lax.dot_general(x_s[p, r0:r0 + nr], w, _NN, preferred_element_type=f32)
        q = pltpu.bitcast((q * SCALE).astype(bf16), u32)
        for c in range(2):
            q_s[2 * h + c, r0 // 2:(r0 + nr) // 2] = q[:, c * 128:(c + 1) * 128]

    def rows(b):
        return pl.ds(pl.multiple_of(b * (SQ // 2), SQ // 2), SQ // 2)

    def ld_q(q_s, b, h):
        return pltpu.bitcast(jnp.concatenate([q_s[2 * h, rows(b)], q_s[2 * h + 1, rows(b)]], axis=1), bf16)

    def st_o(b, h, o):
        o = pltpu.bitcast(o, u32)
        for c in range(2):
            o_s[2 * h + c, rows(b)] = o[:, c * 128:(c + 1) * 128]

    def oproj(h, nh, t, nt):
        r = pl.ds(_mult(t * 64, 64), nt * 64)
        o = jnp.concatenate([o_s[2 * h + i, r] for i in range(2 * nh)], axis=1)
        return lax.dot_general(wo_s[:, pl.ds(_mult(h * DH, DH), nh * DH)], pltpu.bitcast(o, bf16), _NT,
                               preferred_element_type=f32)

    def emit(t, c0, c1):
        out_s[pl.ds(_mult(t * 128, 128), 128), c0:c1] = acc_s[t, c0:c1].T.astype(bf16)

    first, r_done, h_done = [], 0, 0
    for (r, h), s in zip(FIRST, S_FIRST):
        cs, work = [], []
        if r > r_done:
            cs.append(copy(xa.at[pl.ds(r_done, r - r_done)], x_s.at[0, pl.ds(r_done, r - r_done)], s))
            work += [(i, r_done, r - r_done) for i in range(h_done)]
        cs += [c_wq(wqa, WQA, i, s) for i in range(h_done, h)]
        first.append((cs, work + [(i, 0, r) for i in range(h_done, h)]))
        r_done, h_done = r, h
    hp = (H - h_done) // QN
    g_q2 = [c_wq(wqa, WQA, h, S_Q2) for h in range(h_done, h_done + hp)]
    g_q3 = [c_wq(wqa, WQA, h, S_Q3) for h in range(h_done + hp, H)]
    g_xb = [copy(xb, x_s.at[1], S_A)]
    start(sum([cs for cs, _ in first], []) + g_q2 + g_q3 + g_xb + g_a(0, QN * N1 * PR) + g_a(1, NX * PR))

    @pl.loop(0, NTT)
    def _(t):
        acc_s[t] = jnp.zeros((2 * D, 128), f32)

    for k, (cs, work) in enumerate(first):
        wait(cs)
        if k == len(first) - 1:
            start(g_a(2, NX * PR))
        for h, r0, nr in work:
            qproj(0, WQA + h, qa_s, h, r0, nr)
    wait(g_q2)

    @pl.loop(0, QN)
    def _(c):
        @pl.when(c == 1)
        def _():
            start(g_a(3, NX * PR) + [c_kv(kb, pl.ds(0, B), i, t_slot(0, 0, i), 0, NK * PR, S_B) for i in range(2)])
            wait(g_q3)

        ps = pieces(va, [(b, h, a_slot(b, 1, h), S_A) for b in range(2) for h in range(HKV)], N1, k0=c * N1)
        for i in range(hp):
            h = h_done + hp * c + i
            for r0, r1 in zip(MB[:-1], MB[1:]):
                qproj(0, WQA + h, qa_s, h, r0, r1 - r0, ps)
                drip(ps)
        assert not ps

    wait(g_xb)

    g_wob = [c_wo(wob, 4, H + 4, H - 4, S_WO)]

    @pl.loop(0, NA)
    def _(u):
        wait(g_a(u))
        bulk = [c_wo(woa, 4 * u, 4 * u, 4, S_B + u)] + g_t(u, NK * PR, NP * PR)
        un = jnp.minimum(u + 1, NA - 1)
        ps = (pieces(va, [(2 * un + i, h, a_slot(2 * un + i, 1, h), S_A + un) for i in range(2) for h in range(HKV)],
                     NX, u < NA - 1)
              + pieces(vb, [(b, 2 * u + i, t_slot(b, 1, 2 * u + i), S_B + u) for i in range(2) for b in range(B)], NP))
        n, ss = 2 * HKV, {}
        for g in range(n + 1):
            if g < n:
                drip(ps)
                b, kh = 2 * u + g // HKV, g % HKV
                q = jnp.concatenate([ld_q(qa_s, b, 2 * kh + r) for r in range(2)], axis=0)
                ss[g] = lax.dot_general(q, ld_k(a_slot(b, 0, kh), ps), _NT, preferred_element_type=f32)
            i = g - 1
            if i == HKV:
                @pl.when(u == NA - 1)
                def _():
                    start([c_wo(wob, 0, H, 4, S_B + NA)] + g_t(NA, NK * PR, 0) + g_wob
                          + [c_kv(vb, 0, pl.ds(HT, HL), l_slot(0, 1, HT), 0, NV * PR, 0)])
            if i >= 0:
                drip(ps)
                if bulk:
                    start([bulk.pop(0)])
                qproj(1, WQB + 4 * u + i // 4, qb_s, 4 * u + i // 4, (i % 4) * T // 4, T // 4, ps)
                drip(ps)
                b, kh = 2 * u + i // HKV, i % HKV
                o = _pv(ss.pop(i), ld_cols(a_slot(b, 1, kh), SK, ps), True)
                for r in range(2):
                    st_o(b, 2 * kh + r, o[r * SQ:(r + 1) * SQ])
        assert not ps and not bulk

    @pl.loop(0, NB)
    def _(u):
        wait([c_wo(woa, 0, 0, 4, S_B + u)] + g_t(u))
        more = u < NB - 1
        ps = pieces(kb, [(b, 2 * u + 2 + i, jnp.where(more, t_slot(b, 0, 2 * u + 2 + i), l_slot(b, 0, HT + i)),
                          jnp.where(more, S_B + u + 1, b)) for i in range(2) for b in range(B)], NK)
        a0 = pl.multiple_of(jnp.where(u < NA, 0, D), D)
        n, ss, pend = 2 * B, {}, None
        for g in range(n + 1):
            if g < n:
                b, h = g % B, 2 * u + g // B
                ss[g] = lax.dot_general(ld_q(qb_s, b, h), ld_k(t_slot(b, 0, h), ps if g else []), _NT,
                                        preferred_element_type=f32)
                if g > 0:
                    drip(ps)
                if g == 2:
                    @pl.when(u > 1)
                    def _():
                        start(late(2 * u - 4, H, 2 * u - 4) + late(2 * u - 3, H, 2 * u - 3))
            if (n - g) % 2 == 0 and (n - g) // 2 < NTT:
                t = NTT - 1 - (n - g) // 2
                acc_s[t, pl.ds(a0, D)] += oproj(4 * u, 4, t, 1)
            i = g - 1
            if i >= 0:
                drip(ps)
                if pend:
                    st_o(*pend)
                b, h = i % B, 2 * u + i // B
                pend = (b, H + h, _pv(ss.pop(i), ld_cols(t_slot(b, 1, h), SK, ps), False))
        st_o(*pend)
        assert not ps

    h2 = H - LG
    wait(g_wob)
    for b in range(B - 2, B):
        s2 = S_B + 2 * (b - (B - 2))
        start(late(b, h2, b) + [c_kv(kb, b, pl.ds(h2, LG), l_slot(b, 0, h2), 0, SK, s2),
                                c_kv(vb, b, pl.ds(h2, LG), l_slot(b, 1, h2), NV * PR, SK - NV * PR, s2 + 1)])
    emit(NTT - 1, 0, 384)
    d = oproj(H + 4, HT - 4, 0, NTT - 1)
    for t in range(NTT - 1):
        acc_s[t, D:2 * D] += d[:, t * 128:(t + 1) * 128]

    @pl.loop(0, B)
    def _(b):
        split = b >= B - 2
        s2 = S_B + 2 * jnp.maximum(b - (B - 2), 0)
        wait(g_l(b, HT, HL - LG, b))
        pl.when(b < B - 2)(lambda: wait(g_l(b, h2, LG, b)))
        nb = jnp.minimum(b + 1, B - 1)
        vs = jnp.where(nb >= B - 2, S_B + 2 * (nb - (B - 2)) + 1, nb)
        ps = pieces(vb, [(nb, h, l_slot(nb, 1, h), vs if h >= h2 else nb) for h in range(HT, H)], NV, b < B - 1)
        t = jnp.where(b == 0, NTT - 1, b - 1)
        hb = jnp.where(b == 0, H + 4, H + HT)
        ss, pend, acc = {}, None, None
        for g in range(HL + 4):
            if g < HL:
                if g == HL - LG:
                    pl.when(split)(lambda: wait(g_l(b, h2, LG, s2)[:1]))
                    pl.when(b == B - 1)(lambda: start(c_out(0, T - 256, 0, 2 * D) + c_out(T - 128, 128, 0, 384)))
                ss[g] = lax.dot_general(ld_q(qb_s, b, HT + g), ld_k(l_slot(b, 0, HT + g), ps if g else []), _NT,
                                        preferred_element_type=f32)
                if g > 0:
                    drip(ps)
            if g == HL + 1:
                emit(jnp.maximum(b - 2, 0), 0, 2 * D)
            if g == HL + 3:
                st_o(*pend)
            if g >= HL + 1:
                d = oproj(hb + 2 * (g - HL - 1), 2, t, 1)
                acc = d if acc is None else acc + d
            i = g - 2
            if 0 <= i < HL:
                if pend:
                    st_o(*pend)
                if i == HL - LG:
                    pl.when(split)(lambda: wait(g_l(b, h2, LG, s2 + 1)[1:]))
                pend = (b, H + HT + i, _pv(ss.pop(i), ld_cols(l_slot(b, 1, HT + i), SK, ps), True))
                drip(ps)
        acc_s[t, D:2 * D] += acc
        assert not ps

    start(c_out(T - 256, 128, 0, 2 * D), 0)
    for c0 in range(384, 2 * D, 256):
        emit(NTT - 1, c0, c0 + 256)
        start(c_out(T - 128, 128, c0, 256), 0)
    wait(c_out(0, T, 0, 2 * D))


@jax.jit
def pallas_concat_heads__gqa_block_cached__mha_block_cached__near_ridge_kernel(
    A_x: jax.Array,
    A_k_cache: jax.Array,
    A_v_cache: jax.Array,
    A_wq: jax.Array,
    A_wo: jax.Array,
    B_x: jax.Array,
    B_k_cache: jax.Array,
    B_v_cache: jax.Array,
    B_wq: jax.Array,
    B_wo: jax.Array,
):
    assert A_x.shape == B_x.shape == (B, SQ, D)
    assert A_k_cache.shape == (B, HKV, SK, DH) and B_k_cache.shape == (B, H, SK, DH)
    hbm = pl.BlockSpec(memory_space=pltpu.HBM)
    bf16, u32 = jnp.bfloat16, jnp.uint32
    out = pl.pallas_call(
        _kernel,
        in_specs=[hbm] * 10,
        out_specs=hbm,
        out_shape=jax.ShapeDtypeStruct((T, 2 * D), bf16),
        scratch_shapes=[
            pltpu.VMEM((2, T, D), bf16),
            pltpu.VMEM((NSLOT, SK, DH), bf16),
            pltpu.VMEM((D, 2 * H * DH), bf16),
            pltpu.VMEM((2 * H, T // 2, 128), u32),
            pltpu.VMEM((2 * H, T // 2, 128), u32),
            pltpu.VMEM((4 * H, T // 2, 128), u32),
            pltpu.VMEM((NTT, 2 * D, 128), jnp.float32),
            pltpu.VMEM((T, 2 * D), bf16),
            pltpu.SemaphoreType.DMA((NSEM,)),
        ],
        compiler_params=pltpu.CompilerParams(
            vmem_limit_bytes=127 * 2**20,
            disable_bounds_checks=True,
            flags={"XLA_TPU_RESCHEDULE_DMA_DONES": True},
        ),
    )(A_x.reshape(T, D), A_k_cache, A_v_cache, A_wq, A_wo.T,
      B_x.reshape(T, D), B_k_cache, B_v_cache, B_wq, B_wo.T)
    return out.reshape(B, SQ, 2 * D)
```

```python
import functools
import math

import jax
import jax.numpy as jnp
from jax import lax
import jax.experimental.pallas as pl
import jax.experimental.pallas.tpu as pltpu

_NT = (((1,), (1,)), ((), ()))
_NN = (((1,), (0,)), ((), ()))

B, SQ, D, H, HKV, SK, DH = 8, 112, 448, 16, 8, 512, 256
T = B * SQ
NTT = T // 128
NA, NB = 4, 5
HT = 2 * NB
HL = H - HT
LG = 2
SCALE = (DH ** -0.5) * math.log2(math.e)

KV_A, KV_B, WQA, WQB, NSLOT = 0, 2 * B * HKV, 2 * B * (HKV + HT), 2 * B * (HKV + HT) + H, 2 * B * (HKV + HT) + 2 * H
S_A, S_Q2, S_Q3, S_B, S_OUT, S_WO, NSEM = 0, 6, 7, 8, 12, 13, 14
S_FIRST = (4, 5, 9, 10, 11, 12, 13)
FIRST = ((224, 1), (336, 1), (448, 1), (448, 2), (672, 2), (896, 2), (896, 4))
QN = 2
MB = (0, 304, 608, 896)
PR, PRB = 64, 48
N1, NX, NP, NK, NV = 2, 2, 4, 3, 3


def _pv(s, v, normalize_first):
    p = jnp.exp2(s - jnp.max(s, axis=-1, keepdims=True))
    l = jnp.sum(p, axis=-1, keepdims=True)
    r = pl.reciprocal(l, approx=True)
    r = r * (2.0 - l * r)
    if normalize_first:
        o = lax.dot_general((p * r).astype(v.dtype), v, _NN, preferred_element_type=jnp.float32)
    else:
        o = lax.dot_general(p.astype(v.dtype), v, _NN, preferred_element_type=jnp.float32) * r
    return o.astype(v.dtype)


def _mult(i, n):
    return i if isinstance(i, int) else pl.multiple_of(i, n)


def _kernel(xa, ka, va, wqa, woa, xb, kb, vb, wqb, wob, out,
            x_s, pool, wo_s, qa_s, qb_s, o_s, acc_s, out_s, sem):
    f32, bf16, u32 = jnp.float32, jnp.bfloat16, jnp.uint32

    def copy(src, dst, s):
        return lambda: pltpu.make_async_copy(src, dst, sem.at[s])

    def start(cs, priority=1):
        for c in cs:
            c().start(priority=priority)

    def wait(cs):
        for c in cs:
            c().wait()

    def drip(ps):
        if ps:
            cond, c = ps.pop(0)
            if cond is None:
                start([c], 0)
            else:
                pl.when(cond)(functools.partial(start, [c], 0))

    def c_kv(src, b, h, slot, r0, nr, s):
        n = b.size if isinstance(b, pl.Slice) else h.size
        return copy(src.at[b, h, pl.ds(r0, nr)], pool.at[pl.ds(slot, n), pl.ds(r0, nr)], s)

    def pieces(src, tiles, n, cond=None, k0=0, nr=PR):
        return [(cond, c_kv(src, b, pl.ds(h, 1), slot, (k0 + k) * nr, nr, s))
                for b, h, slot, s in tiles for k in range(n)]

    def c_wq(src, base, h, s):
        return copy(src.at[:, pl.ds(_mult(h * DH, DH), DH)], pool.at[base + h, pl.ds(0, D)], s)

    def c_wo(src, h_src, h_dst, n, s):
        return copy(src.at[:, pl.ds(_mult(h_src * DH, DH), n * DH)], wo_s.at[:, pl.ds(_mult(h_dst * DH, DH), n * DH)], s)

    def c_out(r0, nr, c0, nc):
        return [copy(out_s.at[pl.ds(r0, nr), pl.ds(c0, nc)], out.at[pl.ds(r0, nr), pl.ds(c0, nc)], S_OUT)]

    a_slot = lambda b, j, h: KV_A + (b * 2 + j) * HKV + h
    t_slot = lambda b, j, h: KV_B + (h * 2 + j) * B + b
    l_slot = lambda b, j, h: KV_A + (b * 2 + j) * HL + h - HT

    def g_a(u, rv=0):
        cs = [c_wq(wqb, WQB, 4 * u + i, S_A + u) for i in range(4)]
        for b in (2 * u, 2 * u + 1):
            cs += [c_kv(ka, b, pl.ds(0, HKV), a_slot(b, 0, 0), 0, SK, S_A + u),
                   c_kv(va, b, pl.ds(0, HKV), a_slot(b, 1, 0), rv, SK - rv, S_A + u)]
        return cs

    def g_t(u, rk=0, rv=0):
        return [c_kv(src, pl.ds(0, B), 2 * u + i, t_slot(0, j, 2 * u + i), r0, SK - r0, S_B + u)
                for i in range(2) for j, (src, r0) in enumerate(((kb, rk), (vb, rv)))]

    def g_l(b, h0, n, s):
        return [c_kv(src, b, pl.ds(h0, n), l_slot(b, j, h0), 0, SK, s) for j, src in enumerate((kb, vb))]

    def late(b, h1, s):
        return [c_kv(kb, b, pl.ds(HT, 2), l_slot(b, 0, HT), NK * PRB, SK - NK * PRB, s),
                c_kv(kb, b, pl.ds(HT + 2, h1 - HT - 2), l_slot(b, 0, HT + 2), 0, SK, s),
                c_kv(vb, b, pl.ds(HT, h1 - HT), l_slot(b, 1, HT), NV * PRB, SK - NV * PRB, s)]

    def ld_k(slot, ps):
        lo = pool[slot, 0:SK // 2]
        drip(ps)
        return jnp.concatenate([lo, pool[slot, SK // 2:SK]], axis=0)

    def ld_cols(slot, nr, ps):
        lo = pool[slot, 0:nr, 0:128]
        drip(ps)
        return jnp.concatenate([lo, pool[slot, 0:nr, 128:DH]], axis=1)

    def qproj(p, slot, q_s, h, r0, nr, ps=None):
        w = pool[slot, 0:D] if ps is None else ld_cols(slot, D, ps)
        q = lax.dot_general(x_s[p, r0:r0 + nr], w, _NN, preferred_element_type=f32)
        q = pltpu.bitcast((q * SCALE).astype(bf16), u32)
        for c in range(2):
            q_s[2 * h + c, r0 // 2:(r0 + nr) // 2] = q[:, c * 128:(c + 1) * 128]

    def rows(b):
        return pl.ds(pl.multiple_of(b * (SQ // 2), SQ // 2), SQ // 2)

    def ld_q(q_s, b, h):
        return pltpu.bitcast(jnp.concatenate([q_s[2 * h, rows(b)], q_s[2 * h + 1, rows(b)]], axis=1), bf16)

    def st_o(b, h, o):
        o = pltpu.bitcast(o, u32)
        for c in range(2):
            o_s[2 * h + c, rows(b)] = o[:, c * 128:(c + 1) * 128]

    def oproj(h, nh, t, nt):
        r = pl.ds(_mult(t * 64, 64), nt * 64)
        o = jnp.concatenate([o_s[2 * h + i, r] for i in range(2 * nh)], axis=1)
        return lax.dot_general(wo_s[:, pl.ds(_mult(h * DH, DH), nh * DH)], pltpu.bitcast(o, bf16), _NT,
                               preferred_element_type=f32)

    def emit(t, c0, c1):
        out_s[pl.ds(_mult(t * 128, 128), 128), c0:c1] = acc_s[t, c0:c1].T.astype(bf16)

    first, r_done, h_done = [], 0, 0
    for (r, h), s in zip(FIRST, S_FIRST):
        cs, work = [], []
        if r > r_done:
            cs.append(copy(xa.at[pl.ds(r_done, r - r_done)], x_s.at[0, pl.ds(r_done, r - r_done)], s))
            work += [(i, r_done, r - r_done) for i in range(h_done)]
        cs += [c_wq(wqa, WQA, i, s) for i in range(h_done, h)]
        first.append((cs, work + [(i, 0, r) for i in range(h_done, h)]))
        r_done, h_done = r, h
    hp = (H - h_done) // QN
    g_q2 = [c_wq(wqa, WQA, h, S_Q2) for h in range(h_done, h_done + hp)]
    g_q3 = [c_wq(wqa, WQA, h, S_Q3) for h in range(h_done + hp, H)]
    g_xb = [copy(xb, x_s.at[1], S_A)]
    start(sum([cs for cs, _ in first], []) + g_q2 + g_q3 + g_xb + g_a(0, QN * N1 * PR) + g_a(1, NX * PR))

    @pl.loop(0, NTT)
    def _(t):
        acc_s[t] = jnp.zeros((2 * D, 128), f32)

    for k, (cs, work) in enumerate(first):
        wait(cs)
        if k == len(first) - 1:
            start(g_a(2, NX * PR))
        for h, r0, nr in work:
            qproj(0, WQA + h, qa_s, h, r0, nr)
    wait(g_q2)

    @pl.loop(0, QN)
    def _(c):
        @pl.when(c == 1)
        def _():
            start(g_a(3, NX * PR) + [c_kv(kb, pl.ds(0, B), i, t_slot(0, 0, i), 0, NK * PRB, S_B) for i in range(2)])
            wait(g_q3)

        ps = pieces(va, [(b, h, a_slot(b, 1, h), S_A) for b in range(2) for h in range(HKV)], N1, k0=c * N1)
        for i in range(hp):
            h = h_done + hp * c + i
            for r0, r1 in zip(MB[:-1], MB[1:]):
                qproj(0, WQA + h, qa_s, h, r0, r1 - r0, ps)
                drip(ps)
        assert not ps

    wait(g_xb)

    g_wob = [c_wo(wob, 4, H + 4, H - 4, S_WO)]

    @pl.loop(0, NA)
    def _(u):
        wait(g_a(u))
        bulk = [c_wo(woa, 4 * u, 4 * u, 4, S_B + u)] + g_t(u, NK * PRB, NP * PR)
        un = jnp.minimum(u + 1, NA - 1)
        ps = (pieces(va, [(2 * un + i, h, a_slot(2 * un + i, 1, h), S_A + un) for i in range(2) for h in range(HKV)],
                     NX, u < NA - 1)
              + pieces(vb, [(b, 2 * u + i, t_slot(b, 1, 2 * u + i), S_B + u) for i in range(2) for b in range(B)], NP))
        n, ss = 2 * HKV, {}
        for g in range(n + 1):
            if g < n:
                drip(ps)
                b, kh = 2 * u + g // HKV, g % HKV
                q = jnp.concatenate([ld_q(qa_s, b, 2 * kh + r) for r in range(2)], axis=0)
                ss[g] = lax.dot_general(q, ld_k(a_slot(b, 0, kh), ps), _NT, preferred_element_type=f32)
            i = g - 1
            if i == HKV:
                @pl.when(u == NA - 1)
                def _():
                    start([c_wo(wob, 0, H, 4, S_B + NA)] + g_t(NA, NK * PRB, 0) + g_wob
                          + [c_kv(vb, 0, pl.ds(HT, HL), l_slot(0, 1, HT), 0, NV * PRB, 0)])
            if i >= 0:
                drip(ps)
                if bulk:
                    start([bulk.pop(0)])
                qproj(1, WQB + 4 * u + i // 4, qb_s, 4 * u + i // 4, (i % 4) * T // 4, T // 4, ps)
                drip(ps)
                b, kh = 2 * u + i // HKV, i % HKV
                o = _pv(ss.pop(i), ld_cols(a_slot(b, 1, kh), SK, ps), True)
                for r in range(2):
                    st_o(b, 2 * kh + r, o[r * SQ:(r + 1) * SQ])
        assert not ps and not bulk

    @pl.loop(0, NB)
    def _(u):
        wait([c_wo(woa, 4 * jnp.minimum(u, NA - 1), 4 * u, 4, S_B + u)] + g_t(u))
        more = u < NB - 1
        ps = pieces(kb, [(b, 2 * u + 2 + i, jnp.where(more, t_slot(b, 0, 2 * u + 2 + i), l_slot(b, 0, HT + i)),
                          jnp.where(more, S_B + u + 1, b)) for i in range(2) for b in range(B)], NK, nr=PRB)
        a0 = pl.multiple_of(jnp.where(u < NA, 0, D), D)
        n, ss, pend = 2 * B, {}, None
        for g in range(n + 1):
            if g < n:
                b, h = g % B, 2 * u + g // B
                ss[g] = lax.dot_general(ld_q(qb_s, b, h), ld_k(t_slot(b, 0, h), ps if g else []), _NT,
                                        preferred_element_type=f32)
                if g > 0:
                    drip(ps)
                if g == 2:
                    @pl.when(u > 1)
                    def _():
                        start(late(2 * u - 4, H, 2 * u - 4) + late(2 * u - 3, H, 2 * u - 3))
            if (n - g) % 2 == 0 and (n - g) // 2 < NTT:
                t = NTT - 1 - (n - g) // 2
                acc_s[t, pl.ds(a0, D)] += oproj(4 * u, 4, t, 1)
            i = g - 1
            if i >= 0:
                drip(ps)
                if pend:
                    st_o(*pend)
                b, h = i % B, 2 * u + i // B
                pend = (b, H + h, _pv(ss.pop(i), ld_cols(t_slot(b, 1, h), SK, ps), False))
        st_o(*pend)
        assert not ps

    h2 = H - LG
    wait(g_wob)
    for b in range(B - 2, B):
        s2 = S_B + 2 * (b - (B - 2))
        start(late(b, h2, b) + [c_kv(kb, b, pl.ds(h2, LG), l_slot(b, 0, h2), 0, SK, s2),
                                c_kv(vb, b, pl.ds(h2, LG), l_slot(b, 1, h2), NV * PRB, SK - NV * PRB, s2 + 1)])
    emit(NTT - 1, 0, 384)
    d = oproj(H + 4, HT - 4, 0, NTT - 1)
    for t in range(NTT - 1):
        acc_s[t, D:2 * D] += d[:, t * 128:(t + 1) * 128]

    @pl.loop(0, B)
    def _(b):
        split = b >= B - 2
        s2 = S_B + 2 * jnp.maximum(b - (B - 2), 0)
        wait(g_l(b, HT, HL - LG, b))
        pl.when(b < B - 2)(lambda: wait(g_l(b, h2, LG, b)))
        nb = jnp.minimum(b + 1, B - 1)
        vs = jnp.where(nb >= B - 2, S_B + 2 * (nb - (B - 2)) + 1, nb)
        ps = pieces(vb, [(nb, h, l_slot(nb, 1, h), vs if h >= h2 else nb) for h in range(HT, H)], NV,
                    b < B - 1, nr=PRB)
        t = jnp.where(b == 0, NTT - 1, b - 1)
        hb = jnp.where(b == 0, H + 4, H + HT)
        ss, pend, acc = {}, None, None
        for g in range(HL + 4):
            if g < HL:
                if g == HL - LG:
                    pl.when(split)(lambda: wait(g_l(b, h2, LG, s2)[:1]))
                    pl.when(b == B - 1)(lambda: start(c_out(0, T - 256, 0, 2 * D) + c_out(T - 128, 128, 0, 384)))
                ss[g] = lax.dot_general(ld_q(qb_s, b, HT + g), ld_k(l_slot(b, 0, HT + g), ps if g else []), _NT,
                                        preferred_element_type=f32)
                if g > 0:
                    drip(ps)
            if g == HL + 2:
                emit(jnp.maximum(b - 2, 0), 0, 2 * D)
            if g == HL + 3:
                st_o(*pend)
            if g >= HL + 1:
                d = oproj(hb + 2 * (g - HL - 1), 2, t, 1)
                acc = d if acc is None else acc + d
            i = g - 2
            if 0 <= i < HL:
                if pend:
                    st_o(*pend)
                if i == HL - LG:
                    pl.when(split)(lambda: wait(g_l(b, h2, LG, s2 + 1)[1:]))
                pend = (b, H + HT + i, _pv(ss.pop(i), ld_cols(l_slot(b, 1, HT + i), SK, ps), True))
                drip(ps)
        acc_s[t, D:2 * D] += acc
        assert not ps

    start(c_out(T - 256, 128, 0, 2 * D), 0)
    for c0 in range(384, 2 * D, 256):
        emit(NTT - 1, c0, c0 + 256)
        start(c_out(T - 128, 128, c0, 256), 0)
    wait(c_out(0, T, 0, 2 * D))


@jax.jit
def pallas_concat_heads__gqa_block_cached__mha_block_cached__near_ridge_kernel(
    A_x: jax.Array,
    A_k_cache: jax.Array,
    A_v_cache: jax.Array,
    A_wq: jax.Array,
    A_wo: jax.Array,
    B_x: jax.Array,
    B_k_cache: jax.Array,
    B_v_cache: jax.Array,
    B_wq: jax.Array,
    B_wo: jax.Array,
):
    assert A_x.shape == B_x.shape == (B, SQ, D)
    assert A_k_cache.shape == (B, HKV, SK, DH) and B_k_cache.shape == (B, H, SK, DH)
    hbm = pl.BlockSpec(memory_space=pltpu.HBM)
    bf16, u32 = jnp.bfloat16, jnp.uint32
    out = pl.pallas_call(
        _kernel,
        in_specs=[hbm] * 10,
        out_specs=hbm,
        out_shape=jax.ShapeDtypeStruct((T, 2 * D), bf16),
        scratch_shapes=[
            pltpu.VMEM((2, T, D), bf16),
            pltpu.VMEM((NSLOT, SK, DH), bf16),
            pltpu.VMEM((D, 2 * H * DH), bf16),
            pltpu.VMEM((2 * H, T // 2, 128), u32),
            pltpu.VMEM((2 * H, T // 2, 128), u32),
            pltpu.VMEM((4 * H, T // 2, 128), u32),
            pltpu.VMEM((NTT, 2 * D, 128), jnp.float32),
            pltpu.VMEM((T, 2 * D), bf16),
            pltpu.SemaphoreType.DMA((NSEM,)),
        ],
        compiler_params=pltpu.CompilerParams(
            vmem_limit_bytes=127 * 2**20,
            disable_bounds_checks=True,
            flags={"XLA_TPU_RESCHEDULE_DMA_DONES": True},
        ),
    )(A_x.reshape(T, D), A_k_cache, A_v_cache, A_wq, A_wo.T,
      B_x.reshape(T, D), B_k_cache, B_v_cache, B_wq, B_wo.T)
    return out.reshape(B, SQ, 2 * D)
```

```python
import functools
import math

import jax
import jax.numpy as jnp
from jax import lax
import jax.experimental.pallas as pl
import jax.experimental.pallas.tpu as pltpu

_NT = (((1,), (1,)), ((), ()))
_NN = (((1,), (0,)), ((), ()))

B, SQ, D, H, HKV, SK, DH = 8, 112, 448, 16, 8, 512, 256
T = B * SQ
NTT = T // 128
NA, NB = 4, 5
HT = 2 * NB
HL = H - HT
LG = 2
SCALE = (DH ** -0.5) * math.log2(math.e)

KV_A, KV_B, WQA, WQB, NSLOT = 0, 2 * B * HKV, 2 * B * (HKV + HT), 2 * B * (HKV + HT) + H, 2 * B * (HKV + HT) + 2 * H
S_A, S_Q2, S_Q3, S_B, S_OUT, S_WO, NSEM = 0, 6, 7, 8, 12, 13, 14
S_FIRST = (4, 5, 9, 10, 11, 12, 13)
FIRST = ((224, 1), (336, 1), (448, 1), (448, 2), (672, 2), (896, 2), (896, 4))
QN = 2
MB = (0, 304, 608, 896)
PR = 64
N1, NX, NP, NK, NV = 2, 2, 4, 3, 3


def _pv(s, v, normalize_first):
    p = jnp.exp2(s - jnp.max(s, axis=-1, keepdims=True))
    l = jnp.sum(p, axis=-1, keepdims=True)
    r = pl.reciprocal(l, approx=True)
    r = r * (2.0 - l * r)
    if normalize_first:
        o = lax.dot_general((p * r).astype(v.dtype), v, _NN, preferred_element_type=jnp.float32)
    else:
        o = lax.dot_general(p.astype(v.dtype), v, _NN, preferred_element_type=jnp.float32) * r
    return o.astype(v.dtype)


def _mult(i, n):
    return i if isinstance(i, int) else pl.multiple_of(i, n)


def _kernel(xa, ka, va, wqa, woa, xb, kb, vb, wqb, wob, out,
            x_s, pool, wo_s, qa_s, qb_s, o_s, acc_s, out_s, sem):
    f32, bf16, u32 = jnp.float32, jnp.bfloat16, jnp.uint32

    def copy(src, dst, s):
        return lambda: pltpu.make_async_copy(src, dst, sem.at[s])

    def start(cs, priority=1):
        for c in cs:
            c().start(priority=priority)

    def wait(cs):
        for c in cs:
            c().wait()

    def drip(ps):
        if ps:
            cond, c = ps.pop(0)
            if cond is None:
                start([c], 0)
            else:
                pl.when(cond)(functools.partial(start, [c], 0))

    def c_kv(src, b, h, slot, r0, nr, s):
        n = b.size if isinstance(b, pl.Slice) else h.size
        return copy(src.at[b, h, pl.ds(r0, nr)], pool.at[pl.ds(slot, n), pl.ds(r0, nr)], s)

    def pieces(src, tiles, n, cond=None, k0=0):
        return [(cond, c_kv(src, b, pl.ds(h, 1), slot, (k0 + k) * PR, PR, s))
                for b, h, slot, s in tiles for k in range(n)]

    def c_wq(src, base, h, s):
        return copy(src.at[:, pl.ds(_mult(h * DH, DH), DH)], pool.at[base + h, pl.ds(0, D)], s)

    def c_wo(src, h_src, h_dst, n, s):
        return copy(src.at[:, pl.ds(_mult(h_src * DH, DH), n * DH)], wo_s.at[:, pl.ds(_mult(h_dst * DH, DH), n * DH)], s)

    def c_out(r0, nr, c0, nc):
        return [copy(out_s.at[pl.ds(r0, nr), pl.ds(c0, nc)], out.at[pl.ds(r0, nr), pl.ds(c0, nc)], S_OUT)]

    a_slot = lambda b, j, h: KV_A + (b * 2 + j) * HKV + h
    t_slot = lambda b, j, h: KV_B + (h * 2 + j) * B + b
    l_slot = lambda b, j, h: KV_A + (b * 2 + j) * HL + h - HT

    def g_a(u, rv=0):
        cs = [c_wq(wqb, WQB, 4 * u + i, S_A + u) for i in range(4)]
        for b in (2 * u, 2 * u + 1):
            cs += [c_kv(ka, b, pl.ds(0, HKV), a_slot(b, 0, 0), 0, SK, S_A + u),
                   c_kv(va, b, pl.ds(0, HKV), a_slot(b, 1, 0), rv, SK - rv, S_A + u)]
        return cs

    def g_t(u, rk=0, rv=0):
        return [c_kv(src, pl.ds(0, B), 2 * u + i, t_slot(0, j, 2 * u + i), r0, SK - r0, S_B + u)
                for i in range(2) for j, (src, r0) in enumerate(((kb, rk), (vb, rv)))]

    def g_l(b, h0, n, s):
        return [c_kv(src, b, pl.ds(h0, n), l_slot(b, j, h0), 0, SK, s) for j, src in enumerate((kb, vb))]

    def late(b, h1, s):
        return [c_kv(kb, b, pl.ds(HT, 2), l_slot(b, 0, HT), NK * PR, SK - NK * PR, s),
                c_kv(kb, b, pl.ds(HT + 2, h1 - HT - 2), l_slot(b, 0, HT + 2), 0, SK, s),
                c_kv(vb, b, pl.ds(HT, h1 - HT), l_slot(b, 1, HT), NV * PR, SK - NV * PR, s)]

    def ld_k(slot, ps):
        lo = pool[slot, 0:SK // 2]
        drip(ps)
        return jnp.concatenate([lo, pool[slot, SK // 2:SK]], axis=0)

    def ld_cols(slot, nr, ps):
        lo = pool[slot, 0:nr, 0:128]
        drip(ps)
        return jnp.concatenate([lo, pool[slot, 0:nr, 128:DH]], axis=1)

    def qproj(p, slot, q_s, h, r0, nr, ps=None):
        w = pool[slot, 0:D] if ps is None else ld_cols(slot, D, ps)
        q = lax.dot_general(x_s[p, r0:r0 + nr], w, _NN, preferred_element_type=f32)
        q = pltpu.bitcast((q * SCALE).astype(bf16), u32)
        for c in range(2):
            q_s[2 * h + c, r0 // 2:(r0 + nr) // 2] = q[:, c * 128:(c + 1) * 128]

    def rows(b):
        return pl.ds(pl.multiple_of(b * (SQ // 2), SQ // 2), SQ // 2)

    def ld_q(q_s, b, h):
        return pltpu.bitcast(jnp.concatenate([q_s[2 * h, rows(b)], q_s[2 * h + 1, rows(b)]], axis=1), bf16)

    def st_o(b, h, o):
        o = pltpu.bitcast(o, u32)
        for c in range(2):
            o_s[2 * h + c, rows(b)] = o[:, c * 128:(c + 1) * 128]

    def oproj(h, nh, t, nt):
        r = pl.ds(_mult(t * 64, 64), nt * 64)
        o = jnp.concatenate([o_s[2 * h + i, r] for i in range(2 * nh)], axis=1)
        return lax.dot_general(wo_s[:, pl.ds(_mult(h * DH, DH), nh * DH)], pltpu.bitcast(o, bf16), _NT,
                               preferred_element_type=f32)

    def emit(t, c0, c1):
        out_s[pl.ds(_mult(t * 128, 128), 128), c0:c1] = acc_s[t, c0:c1].T.astype(bf16)

    first, r_done, h_done = [], 0, 0
    for (r, h), s in zip(FIRST, S_FIRST):
        cs, work = [], []
        if r > r_done:
            cs.append(copy(xa.at[pl.ds(r_done, r - r_done)], x_s.at[0, pl.ds(r_done, r - r_done)], s))
            work += [(i, r_done, r - r_done) for i in range(h_done)]
        cs += [c_wq(wqa, WQA, i, s) for i in range(h_done, h)]
        first.append((cs, work + [(i, 0, r) for i in range(h_done, h)]))
        r_done, h_done = r, h
    hp = (H - h_done) // QN
    g_q2 = [c_wq(wqa, WQA, h, S_Q2) for h in range(h_done, h_done + hp)]
    g_q3 = [c_wq(wqa, WQA, h, S_Q3) for h in range(h_done + hp, H)]
    g_xb = [copy(xb, x_s.at[1], S_A)]
    start(sum([cs for cs, _ in first], []) + g_q2 + g_q3 + g_xb + g_a(0, QN * N1 * PR) + g_a(1, NX * PR))

    @pl.loop(0, NTT)
    def _(t):
        acc_s[t] = jnp.zeros((2 * D, 128), f32)

    for k, (cs, work) in enumerate(first):
        wait(cs)
        if k == len(first) - 1:
            start(g_a(2, NX * PR))
        for h, r0, nr in work:
            qproj(0, WQA + h, qa_s, h, r0, nr)
    wait(g_q2)

    @pl.loop(0, QN)
    def _(c):
        @pl.when(c == 1)
        def _():
            start(g_a(3, NX * PR) + [c_kv(kb, pl.ds(0, B), i, t_slot(0, 0, i), 0, NK * PR, S_B) for i in range(2)])
            wait(g_q3)

        ps = pieces(va, [(b, h, a_slot(b, 1, h), S_A) for b in range(2) for h in range(HKV)], N1, k0=c * N1)
        for i in range(hp):
            h = h_done + hp * c + i
            for r0, r1 in zip(MB[:-1], MB[1:]):
                qproj(0, WQA + h, qa_s, h, r0, r1 - r0, ps)
                drip(ps)
        assert not ps

    wait(g_xb)

    g_wob = [c_wo(wob, 4, H + 4, H - 4, S_WO)]

    @pl.loop(0, NA)
    def _(u):
        wait(g_a(u))
        bulk = [c_wo(woa, 4 * u, 4 * u, 4, S_B + u)] + g_t(u, NK * PR, NP * PR)
        un = jnp.minimum(u + 1, NA - 1)
        ps = (pieces(va, [(2 * un + i, h, a_slot(2 * un + i, 1, h), S_A + un) for i in range(2) for h in range(HKV)],
                     NX, u < NA - 1)
              + pieces(vb, [(b, 2 * u + i, t_slot(b, 1, 2 * u + i), S_B + u) for i in range(2) for b in range(B)], NP))
        n, ss = 2 * HKV, {}
        for g in range(n + 1):
            if g < n:
                drip(ps)
                b, kh = 2 * u + g // HKV, g % HKV
                q = jnp.concatenate([ld_q(qa_s, b, 2 * kh + r) for r in range(2)], axis=0)
                ss[g] = lax.dot_general(q, ld_k(a_slot(b, 0, kh), ps), _NT, preferred_element_type=f32)
            i = g - 1
            if i == HKV:
                @pl.when(u == NA - 1)
                def _():
                    start([c_wo(wob, 0, H, 4, S_B + NA)] + g_t(NA, NK * PR, 0) + g_wob
                          + [c_kv(vb, 0, pl.ds(HT, HL), l_slot(0, 1, HT), 0, NV * PR, 0)])
            if i >= 0:
                drip(ps)
                if bulk:
                    start([bulk.pop(0)])
                qproj(1, WQB + 4 * u + i // 4, qb_s, 4 * u + i // 4, (i % 4) * T // 4, T // 4, ps)
                drip(ps)
                b, kh = 2 * u + i // HKV, i % HKV
                o = _pv(ss.pop(i), ld_cols(a_slot(b, 1, kh), SK, ps), True)
                for r in range(2):
                    st_o(b, 2 * kh + r, o[r * SQ:(r + 1) * SQ])
        assert not ps and not bulk

    @pl.loop(0, NB)
    def _(u):
        wait([c_wo(woa, 4 * jnp.minimum(u, NA - 1), 4 * u, 4, S_B + u)] + g_t(u))
        more = u < NB - 1
        ps = pieces(kb, [(b, 2 * u + 2 + i, jnp.where(more, t_slot(b, 0, 2 * u + 2 + i), l_slot(b, 0, HT + i)),
                          jnp.where(more, S_B + u + 1, b)) for i in range(2) for b in range(B)], NK)
        a0 = pl.multiple_of(jnp.where(u < NA, 0, D), D)
        n, ss, pend = 2 * B, {}, None
        for g in range(n + 1):
            if g < n:
                b, h = g % B, 2 * u + g // B
                ss[g] = lax.dot_general(ld_q(qb_s, b, h), ld_k(t_slot(b, 0, h), ps if g else []), _NT,
                                        preferred_element_type=f32)
                if g > 0:
                    drip(ps)
                if g == 2:
                    @pl.when(u > 1)
                    def _():
                        start(late(2 * u - 4, H, 2 * u - 4) + late(2 * u - 3, H, 2 * u - 3))
            if (n - g) % 2 == 0 and (n - g) // 2 < NTT:
                t = NTT - 1 - (n - g) // 2
                acc_s[t, pl.ds(a0, D)] += oproj(4 * u, 4, t, 1)
            i = g - 1
            if i >= 0:
                drip(ps)
                if pend:
                    st_o(*pend)
                b, h = i % B, 2 * u + i // B
                pend = (b, H + h, _pv(ss.pop(i), ld_cols(t_slot(b, 1, h), SK, ps), False))
        st_o(*pend)
        assert not ps

    h2 = H - LG
    wait(g_wob)
    for b in range(B - 2, B):
        s2 = S_B + 2 * (b - (B - 2))
        start(late(b, h2, b) + [c_kv(kb, b, pl.ds(h2, LG), l_slot(b, 0, h2), 0, SK, s2),
                                c_kv(vb, b, pl.ds(h2, LG), l_slot(b, 1, h2), NV * PR, SK - NV * PR, s2 + 1)])
    emit(NTT - 1, 0, 384)
    d = oproj(H + 4, HT - 4, 0, NTT - 1)
    for t in range(NTT - 1):
        acc_s[t, D:2 * D] += d[:, t * 128:(t + 1) * 128]

    @pl.loop(0, B)
    def _(b):
        split = b >= B - 2
        s2 = S_B + 2 * jnp.maximum(b - (B - 2), 0)
        wait(g_l(b, HT, HL - LG, b))
        pl.when(b < B - 2)(lambda: wait(g_l(b, h2, LG, b)))
        nb = jnp.minimum(b + 1, B - 1)
        vs = jnp.where(nb >= B - 2, S_B + 2 * (nb - (B - 2)) + 1, nb)
        ps = pieces(vb, [(nb, h, l_slot(nb, 1, h), vs if h >= h2 else nb) for h in range(HT, H)], NV, b < B - 1)
        t = jnp.where(b == 0, NTT - 1, b - 1)
        hb = jnp.where(b == 0, H + 4, H + HT)
        ss, pend, acc = {}, None, None
        for g in range(HL + 4):
            if g < HL:
                if g == HL - LG:
                    pl.when(split)(lambda: wait(g_l(b, h2, LG, s2)[:1]))
                    pl.when(b == B - 1)(lambda: start(c_out(0, T - 256, 0, 2 * D) + c_out(T - 128, 128, 0, 384)))
                ss[g] = lax.dot_general(ld_q(qb_s, b, HT + g), ld_k(l_slot(b, 0, HT + g), ps if g else []), _NT,
                                        preferred_element_type=f32)
                if g > 0:
                    drip(ps)
            if g == HL + 2:
                emit(jnp.maximum(b - 2, 0), 0, 2 * D)
            if g == HL + 3:
                st_o(*pend)
            if g >= HL + 1:
                d = oproj(hb + 2 * (g - HL - 1), 2, t, 1)
                acc = d if acc is None else acc + d
            i = g - 2
            if 0 <= i < HL:
                if pend:
                    st_o(*pend)
                if i == HL - LG:
                    pl.when(split)(lambda: wait(g_l(b, h2, LG, s2 + 1)[1:]))
                pend = (b, H + HT + i, _pv(ss.pop(i), ld_cols(l_slot(b, 1, HT + i), SK, ps), True))
                drip(ps)
        acc_s[t, D:2 * D] += acc
        assert not ps

    start(c_out(T - 256, 128, 0, 2 * D), 0)
    for c0 in range(384, 2 * D, 256):
        emit(NTT - 1, c0, c0 + 256)
        start(c_out(T - 128, 128, c0, 256), 0)
    wait(c_out(0, T, 0, 2 * D))


@jax.jit
def pallas_concat_heads__gqa_block_cached__mha_block_cached__near_ridge_kernel(
    A_x: jax.Array,
    A_k_cache: jax.Array,
    A_v_cache: jax.Array,
    A_wq: jax.Array,
    A_wo: jax.Array,
    B_x: jax.Array,
    B_k_cache: jax.Array,
    B_v_cache: jax.Array,
    B_wq: jax.Array,
    B_wo: jax.Array,
):
    assert A_x.shape == B_x.shape == (B, SQ, D)
    assert A_k_cache.shape == (B, HKV, SK, DH) and B_k_cache.shape == (B, H, SK, DH)
    hbm = pl.BlockSpec(memory_space=pltpu.HBM)
    bf16, u32 = jnp.bfloat16, jnp.uint32
    out = pl.pallas_call(
        _kernel,
        in_specs=[hbm] * 10,
        out_specs=hbm,
        out_shape=jax.ShapeDtypeStruct((T, 2 * D), bf16),
        scratch_shapes=[
            pltpu.VMEM((2, T, D), bf16),
            pltpu.VMEM((NSLOT, SK, DH), bf16),
            pltpu.VMEM((D, 2 * H * DH), bf16),
            pltpu.VMEM((2 * H, T // 2, 128), u32),
            pltpu.VMEM((2 * H, T // 2, 128), u32),
            pltpu.VMEM((4 * H, T // 2, 128), u32),
            pltpu.VMEM((NTT, 2 * D, 128), jnp.float32),
            pltpu.VMEM((T, 2 * D), bf16),
            pltpu.SemaphoreType.DMA((NSEM,)),
        ],
        compiler_params=pltpu.CompilerParams(
            vmem_limit_bytes=127 * 2**20,
            disable_bounds_checks=True,
            flags={"XLA_TPU_RESCHEDULE_DMA_DONES": True},
        ),
    )(A_x.reshape(T, D), A_k_cache, A_v_cache, A_wq, A_wo.T,
      B_x.reshape(T, D), B_k_cache, B_v_cache, B_wq, B_wo.T)
    return out.reshape(B, SQ, 2 * D)
```
